```python
import os as _os
_os.environ.setdefault("JAX_PLATFORMS", "cpu")
import jax
import jax.numpy as jnp

def _softmax(x, axis=-1):
    return jax.nn.softmax(x, axis=axis)
def _gelu(x):
    return jax.nn.gelu(x, approximate=True)
def _silu(x):
    return jax.nn.silu(x)
def _sigmoid(x):
    return jax.nn.sigmoid(x)
def _layernorm(x, axis=-1, eps=1e-5):
    m = jnp.mean(x, axis=axis, keepdims=True)
    v = jnp.var(x, axis=axis, keepdims=True)
    return (x - m) / jnp.sqrt(v + eps)
def _scatter_add(tgt, idx, src, axis=0):
    return tgt.at[idx].add(src)
def _segment_sum(src, seg, n):
    return jax.ops.segment_sum(src, seg, n)
class _Rng:
    def __init__(self, key):
        self._k = key
    def _next(self):
        self._k, sub = jax.random.split(self._k)
        return sub
    def normal(self, shape):
        return jax.random.normal(self._next(), shape, dtype=jnp.bfloat16)
    def randint(self, lo, hi, shape):
        return jax.random.randint(self._next(), shape, lo, hi, dtype=jnp.int32)
    def uniform(self, shape, lo=0.0, hi=1.0):
        return jax.random.uniform(self._next(), shape, jnp.bfloat16, lo, hi)
    def permutation(self, n):
        return jax.random.permutation(self._next(), n)


kernel_name = 'interleave_layers__sliding_block__mha_block__prompt'

def setup_inputs():
    _rng = _Rng(jax.random.key(int.from_bytes(__import__("os").urandom(4), "little")))
    _w = (lambda a: (lambda t: t.astype(jnp.bfloat16) if jnp.issubdtype(t.dtype, jnp.floating) else t)(jnp.asarray(a)))
    def _A_setup():
        B, S, D = 1, 2048, 512
        return {
            "x": _w((lambda *s: _rng.normal(s) * 0.05)(B, S, D)),
            "wqkv": _w((lambda *s: _rng.normal(s) * 0.05)(D, 3 * D)),
            "wo": _w((lambda *s: _rng.normal(s) * 0.05)(D, D)),
        }
    _A_in = _A_setup()

    def _B_setup():
        B, S, D, H = 1, 2048, 512, 32
        return {
            "x": _w((lambda *s: _rng.normal(s) * 0.05)(B, S, D)),
            "wqkv": _w((lambda *s: _rng.normal(s) * 0.05)(D, 3 * D)),
            "wo": _w((lambda *s: _rng.normal(s) * 0.05)(D, D)),
        }
    _B_in = _B_setup()

    return {
        "A_x": _A_in["x"],
        "A_wqkv": _A_in["wqkv"],
        "A_wo": _A_in["wo"],
        "B_x": _B_in["x"],
        "B_wqkv": _B_in["wqkv"],
        "B_wo": _B_in["wo"],
    }

def reference(A_x, A_wqkv, A_wo, B_x, B_wqkv, B_wo):
    def _A_ref(x, wqkv, wo):
        B, S, D = x.shape
        H = 32; Dh = D // H; W = 256
        qkv = (lambda x, *d: x.transpose(*d))((x @ wqkv).reshape(B, S, 3, H, Dh), 2, 0, 3, 1, 4)
        q, k, v = qkv[0], qkv[1], qkv[2]
        scores = jnp.einsum("bhqd,bhkd->bhqk", q, k) * (Dh ** -0.5)
        idx = jnp.arange(S)
        mask = (idx[:, None] - idx[None, :] >= 0) & (idx[:, None] - idx[None, :] < W)
        scores = jnp.where(mask[None, None], scores, -1e9)
        p = _softmax(scores, axis=-1)
        o = jnp.einsum("bhqk,bhkd->bhqd", p, v)
        return (lambda x, *d: x.transpose(*d))(o, 0, 2, 1, 3).reshape(B, S, D) @ wo

    def _B_ref(x, wqkv, wo):
        B, S, D = x.shape
        H = 32
        Dh = D // H
        qkv = (lambda x, *d: x.transpose(*d))((x @ wqkv).reshape(B, S, 3, H, Dh), 2, 0, 3, 1, 4)
        q, k, v = qkv[0], qkv[1], qkv[2]
        scores = jnp.einsum("bhqd,bhkd->bhqk", q, k) * (Dh ** -0.5)
        p = _softmax(scores, axis=-1)
        o = jnp.einsum("bhqk,bhkd->bhqd", p, v)
        return (lambda x, *d: x.transpose(*d))(o, 0, 2, 1, 3).reshape(B, S, D) @ wo

    x = A_x
    x = x + _A_ref(_layernorm(x, axis=-1), A_wqkv, A_wo)
    x = x + _B_ref(_layernorm(x, axis=-1), B_wqkv, B_wo)
    x = x + _A_ref(_layernorm(x, axis=-1), A_wqkv, A_wo)
    x = x + _B_ref(_layernorm(x, axis=-1), B_wqkv, B_wo)
    return x
```

```python
import functools
import math

import jax
import jax.numpy as jnp
from jax import lax
import jax.experimental.pallas as pl
import jax.experimental.pallas.tpu as pltpu

S = 2048
D = 512
H = 32
DH = D // H
WIN = 256
LANE = 128
GROUP = LANE // DH
QSCALE = (DH ** -0.5) * math.log2(math.e)
LN_EPS = 1e-5
L_LO = 2.0 ** -40
L_HI = 2.0 ** 40

TM = 512
F32 = jnp.float32
BF16 = jnp.bfloat16


def _head_weights(qt_blk, r):
    q32 = pltpu.bitcast(qt_blk, jnp.uint32)
    rows = lax.broadcasted_iota(jnp.int32, q32.shape, 0) // (DH // 2)
    return pltpu.bitcast(jnp.where(rows == r, q32, jnp.uint32(0)), BF16)


def _bad_flag(l, o):
    ok = jnp.logical_and(l >= L_LO, l <= L_HI)
    omax = jnp.max(jnp.abs(o), axis=0, keepdims=True)
    ok = jnp.logical_and(ok, omax < jnp.inf)
    return jnp.where(ok, 0.0, 1.0)


def _full_attention(k_ref, qt_ref, vt_ref, ot_ref):
    TQ, CK, SKEW, NSUB = 512, 128, 2, 4
    NC = S // CK

    def body(h, bad):
        g0 = pl.multiple_of((h // GROUP) * LANE, LANE)
        r = h % GROUP
        h0 = pl.multiple_of(h * DH, DH)
        ws = [_head_weights(qt_ref[pl.ds(g0, LANE), pl.ds(sub * TQ, TQ)], r)
              for sub in range(NSUB)]
        steps = [(sub, c) for sub in range(NSUB) for c in range(NC)]
        accs = [None] * NSUB
        lsums = [None] * NSUB
        ps = {}
        flags = [bad]

        def qk(sub, c):
            kc = k_ref[pl.ds(c * CK, CK), pl.ds(g0, LANE)]
            s = jnp.dot(kc, ws[sub], preferred_element_type=F32)
            p = jnp.exp2(s)
            part = jnp.sum(p.reshape(CK // 8, 8, TQ), axis=0)
            lsums[sub] = part if c == 0 else lsums[sub] + part
            ps[(sub, c)] = p.astype(BF16)

        def pv(sub, c):
            vt = vt_ref[pl.ds(h0, DH), pl.ds(c * CK, CK)]
            o = jnp.dot(vt, ps.pop((sub, c)), preferred_element_type=F32)
            accs[sub] = o if c == 0 else accs[sub] + o
            if c == NC - 1:
                l = jnp.sum(lsums[sub], axis=0, keepdims=True)
                o = accs[sub] * (1.0 / l)
                ot_ref[pl.ds(h0, DH), pl.ds(sub * TQ, TQ)] = o.astype(BF16)
                flags[0] = jnp.maximum(flags[0], _bad_flag(l, o))

        n = len(steps)
        for i in range(n + SKEW):
            if i < n:
                qk(*steps[i])
            if i >= SKEW:
                pv(*steps[i - SKEW])
        return flags[0]

    return lax.fori_loop(0, H, body, jnp.zeros((1, TQ), F32))


def _sliding_attention(k_ref, qt_ref, vt_ref, ot_ref):
    NH, SKEW = 4, 2
    NB = S // LANE
    NW = WIN // LANE

    def body(it, bad):
        g0 = pl.multiple_of((it // 2) * LANE, LANE)
        r0 = (it % 2) * NH
        hbase = it * NH
        row = lax.broadcasted_iota(jnp.int32, (LANE, NH * LANE), 0)
        col = lax.broadcasted_iota(jnp.int32, (LANE, NH * LANE), 1) % LANE
        steps = [(j, c) for j in range(NB) for c in range(max(0, j - NW), j + 1)]
        ws, accs, lsums, ps = {}, {}, {}, {}
        flags = [bad]

        def qk(j, c):
            first = c == max(0, j - NW)
            if first:
                qt = qt_ref[pl.ds(g0, LANE), pl.ds(j * LANE, LANE)]
                ws[j] = jnp.concatenate(
                    [_head_weights(qt, r0 + u) for u in range(NH)], axis=1)
            kc = k_ref[pl.ds(c * LANE, LANE), pl.ds(g0, LANE)]
            s = jnp.dot(kc, ws[j], preferred_element_type=F32)
            p = jnp.exp2(s)
            if c == j:
                p = jnp.where(row <= col, p, 0.0)
            elif c == j - NW:
                p = jnp.where(row > col, p, 0.0)
            part = jnp.sum(p.reshape(LANE // 8, 8, NH * LANE), axis=0)
            lsums[j] = part if first else lsums[j] + part
            ps[(j, c)] = p.astype(BF16)

        def pv(j, c):
            first = c == max(0, j - NW)
            p = ps.pop((j, c))
            os = []
            for u in range(NH):
                h0 = pl.multiple_of((hbase + u) * DH, DH)
                vt = vt_ref[pl.ds(h0, DH), pl.ds(c * LANE, LANE)]
                os.append(jnp.dot(vt, p[:, u * LANE:(u + 1) * LANE],
                                  preferred_element_type=F32))
            o = jnp.concatenate(os, axis=1)
            accs[j] = o if first else accs[j] + o
            if c == j:
                l = jnp.sum(lsums.pop(j), axis=0, keepdims=True)
                o = accs.pop(j) * (1.0 / l)
                ob = o.astype(BF16)
                for u in range(NH):
                    h0 = pl.multiple_of((hbase + u) * DH, DH)
                    ot_ref[pl.ds(h0, DH), pl.ds(j * LANE, LANE)] = (
                        ob[:, u * LANE:(u + 1) * LANE])
                flags[0] = jnp.maximum(flags[0], _bad_flag(l, o))

        n = len(steps)
        for i in range(n + SKEW):
            if i < n:
                qk(*steps[i])
            if i >= SKEW:
                pv(*steps[i - SKEW])
        return flags[0]

    return lax.fori_loop(0, H // NH, body, jnp.zeros((1, NH * LANE), F32))


def _safe_attention(k_ref, qt_ref, vt_ref, ot_ref, sliding):
    NB = S // LANE
    NK = (WIN + LANE) if sliding else S

    def body(it, carry):
        h = it // NB
        j = it % NB
        g0 = pl.multiple_of((h // GROUP) * LANE, LANE)
        h0 = pl.multiple_of(h * DH, DH)
        q0 = pl.multiple_of(j * LANE, LANE)
        if sliding:
            k0 = pl.multiple_of(jnp.maximum(q0 - WIN, 0), LANE)
        else:
            k0 = 0
        w = _head_weights(qt_ref[pl.ds(g0, LANE), pl.ds(q0, LANE)], h % GROUP)
        kc = k_ref[pl.ds(k0, NK), pl.ds(g0, LANE)]
        s = jnp.dot(kc, w, preferred_element_type=F32)
        if sliding:
            kpos = k0 + lax.broadcasted_iota(jnp.int32, s.shape, 0)
            qpos = q0 + lax.broadcasted_iota(jnp.int32, s.shape, 1)
            d = qpos - kpos
            s = jnp.where(jnp.logical_and(d >= 0, d < WIN), s, -1e9)
        m = jnp.max(s, axis=0, keepdims=True)
        p = jnp.exp2(s - m)
        l = jnp.sum(p, axis=0, keepdims=True)
        p = (p * (1.0 / l)).astype(BF16)
        vt = vt_ref[pl.ds(h0, DH), pl.ds(k0, NK)]
        o = jnp.dot(vt, p, preferred_element_type=F32)
        ot_ref[pl.ds(h0, DH), pl.ds(q0, LANE)] = o.astype(BF16)
        return carry

    lax.fori_loop(0, H * NB, body, 0)


def _attention(k_ref, qt_ref, vt_ref, ot_ref, sliding):
    fast = _sliding_attention if sliding else _full_attention
    bad = fast(k_ref, qt_ref, vt_ref, ot_ref)

    @pl.when(jnp.max(bad) > 0.0)
    def _():
        _safe_attention(k_ref, qt_ref, vt_ref, ot_ref, sliding)


def _project_in(x, r0, wqkv_ref, wt_ref, k_ref, qt_ref, vt_ref):
    m = jnp.mean(x, axis=-1, keepdims=True)
    xc = x - m
    v = jnp.mean(xc * xc, axis=-1, keepdims=True)
    xn = (xc * lax.rsqrt(v + LN_EPS)).astype(BF16)
    k = jnp.dot(xn, wqkv_ref[:, D:2 * D], preferred_element_type=F32)
    k_ref[pl.ds(r0, TM), :] = k.astype(BF16)
    qv = lax.dot_general(wt_ref[...], xn, (((1,), (1,)), ((), ())),
                         preferred_element_type=F32)
    qt_ref[:, pl.ds(r0, TM)] = (qv[:D] * QSCALE).astype(BF16)
    vt_ref[:, pl.ds(r0, TM)] = qv[D:].astype(BF16)


def _project_out(r0, ot_ref, wo_ref):
    ot = ot_ref[:, pl.ds(r0, TM)]
    return lax.dot_general(ot, wo_ref[...], (((0,), (0,)), ((), ())),
                           preferred_element_type=F32)


def _kernel(x_ref, wa_ref, woa_ref, wb_ref, wob_ref, o_ref,
            xres_ref, k_ref, qt_ref, vt_ref, ot_ref, wta_ref, wtb_ref):
    for w_ref, wt_ref in ((wa_ref, wta_ref), (wb_ref, wtb_ref)):
        wt_ref[0:D, :] = w_ref[:, 0:D].astype(F32).T.astype(BF16)
        wt_ref[D:2 * D, :] = w_ref[:, 2 * D:3 * D].astype(F32).T.astype(BF16)

    nchunk = S // TM

    def first_in(i, carry):
        r0 = pl.multiple_of(i * TM, TM)
        x = x_ref[pl.ds(r0, TM), :].astype(F32)
        xres_ref[pl.ds(r0, TM), :] = x
        _project_in(x, r0, wa_ref, wta_ref, k_ref, qt_ref, vt_ref)
        return carry

    def out_in(wo_ref, w_ref, wt_ref):
        def fn(i, carry):
            r0 = pl.multiple_of(i * TM, TM)
            x = xres_ref[pl.ds(r0, TM), :] + _project_out(r0, ot_ref, wo_ref)
            xres_ref[pl.ds(r0, TM), :] = x
            _project_in(x, r0, w_ref, wt_ref, k_ref, qt_ref, vt_ref)
            return carry
        return fn

    def last_out(i, carry):
        r0 = pl.multiple_of(i * TM, TM)
        x = xres_ref[pl.ds(r0, TM), :] + _project_out(r0, ot_ref, wob_ref)
        o_ref[pl.ds(r0, TM), :] = x.astype(o_ref.dtype)
        return carry

    lax.fori_loop(0, nchunk, first_in, 0)

    def pair(t, carry):
        _attention(k_ref, qt_ref, vt_ref, ot_ref, sliding=True)
        lax.fori_loop(0, nchunk, out_in(woa_ref, wb_ref, wtb_ref), 0)
        _attention(k_ref, qt_ref, vt_ref, ot_ref, sliding=False)

        @pl.when(t == 0)
        def _():
            lax.fori_loop(0, nchunk, out_in(wob_ref, wa_ref, wta_ref), 0)
        return carry

    lax.fori_loop(0, 2, pair, 0)
    lax.fori_loop(0, nchunk, last_out, 0)


@jax.jit
def pallas_interleave_layers__sliding_block__mha_block__prompt_kernel(
    A_x: jax.Array,
    A_wqkv: jax.Array,
    A_wo: jax.Array,
    B_x: jax.Array,
    B_wqkv: jax.Array,
    B_wo: jax.Array,
):
    del B_x
    x = A_x.reshape(S, D)
    out = pl.pallas_call(
        _kernel,
        out_shape=jax.ShapeDtypeStruct((S, D), A_x.dtype),
        scratch_shapes=[
            pltpu.VMEM((S, D), F32),
            pltpu.VMEM((S, D), BF16),
            pltpu.VMEM((D, S), BF16),
            pltpu.VMEM((D, S), BF16),
            pltpu.VMEM((D, S), BF16),
            pltpu.VMEM((2 * D, D), BF16),
            pltpu.VMEM((2 * D, D), BF16),
        ],
        compiler_params=pltpu.CompilerParams(vmem_limit_bytes=100 * 1024 * 1024),
    )(x, A_wqkv, A_wo, B_wqkv, B_wo)
    return out.reshape(A_x.shape)
```

```python
import math

import jax
import jax.numpy as jnp
from jax import lax
import jax.experimental.pallas as pl
import jax.experimental.pallas.tpu as pltpu

S = 2048
D = 512
H = 32
DH = D // H
WIN = 256
LANE = 128
GROUP = LANE // DH
NG = D // LANE
NB = S // LANE
QSCALE = (DH ** -0.5) * math.log2(math.e)
LN_EPS = 1e-5
L_LO = 2.0 ** -40
L_HI = 2.0 ** 40

TM = 512
RV = 16
F32 = jnp.float32
BF16 = jnp.bfloat16
U32 = jnp.uint32


def _cat(xs, axis):
    return xs[0] if len(xs) == 1 else jnp.concatenate(xs, axis=axis)


def _pk(x):
    return pltpu.bitcast(x, U32)


def _unpk(x):
    return pltpu.bitcast(x, BF16)


def _head_weights(q32, r):
    rows = lax.broadcasted_iota(jnp.int32, q32.shape, 0) >> 3
    return pltpu.bitcast(jnp.where(rows == r, q32, jnp.uint32(0)), BF16)


def _bad_flag(l, o):
    ok = jnp.logical_and(l >= L_LO, l <= L_HI)
    omax = jnp.max(jnp.abs(o), axis=0, keepdims=True)
    ok = jnp.logical_and(ok, omax < jnp.inf)
    return jnp.where(ok, 0.0, 1.0)


def _mo(x, m):
    return x if isinstance(x, int) else pl.multiple_of(x, m)


def _prep_kb(h, k_ref, kb_ref, c0=0, nc=NB):
    kk = _cat([k_ref[h >> 3, pl.ds(_mo((c0 + c) * (LANE // 2) + (LANE - RV) // 2, 8), RV // 2), :]
               for c in range(nc)], 0)
    if not (isinstance(h, int) and h % GROUP == 0):
        kk = pltpu.roll(kk, (LANE - (h & (GROUP - 1)) * DH) & (LANE - 1), 1)
    for d in range(DH):
        kb_ref[d, pl.ds(_mo(c0 * (RV // 2), 8), nc * (RV // 2)), :] = (
            jnp.broadcast_to(kk[:, d:d + 1], kk.shape))


def _full_attention(k_ref, qt_ref, vt_ref, ot_ref, kb_ref, z_ref):
    NT, SKEW = 4, 2
    TQ = NT * LANE
    NSUB = NB // NT
    nm, nv = (LANE - RV) // 8, RV // 8

    def body(h, bad):
        g = h >> 3
        g0 = pl.multiple_of(g * (LANE // 2), LANE // 2)
        r = h & (GROUP - 1)
        h0 = pl.multiple_of(h * (DH // 2), DH // 2)
        steps = [(sub, c) for sub in range(NSUB) for c in range(NB)]
        ws, qbs, kbs, accs, lsums, ps = {}, {}, {}, {}, {}, {}
        flags = [bad]

        def qk(sub, c):
            if c == 0:
                blks = range(sub * NT, (sub + 1) * NT)
                ws[sub] = _head_weights(
                    _cat([qt_ref[j, pl.ds(g0, LANE // 2), :] for j in blks], 1), r)
                qh = _unpk(_cat([qt_ref[j, pl.ds(h0, DH // 2), :] for j in blks], 1)).astype(F32)
                qbs[sub] = [jnp.broadcast_to(qh[d:d + 1, :], (8, TQ)) for d in range(DH)]
                lsums[sub] = [None] * NT
            if sub == 0:
                kbs[c] = [pltpu.bitcast(kb_ref[d, pl.ds(c * (RV // 2), RV // 2), :],
                                        BF16).astype(F32) for d in range(DH)]
                if c == NB - 1:
                    _prep_kb(jnp.minimum(h + 1, H - 1), k_ref, kb_ref)
            kc = _unpk(k_ref[g, pl.ds(c * (LANE // 2), (LANE - RV) // 2), :])
            s = jnp.dot(kc, ws[sub], preferred_element_type=F32)
            sv = None
            for d in range(DH):
                t = _cat([kbs[c][d]] * NT, 1) * _cat([qbs[sub][d]] * nv, 0)
                sv = t if sv is None else sv + t
            p = jnp.exp2(jnp.concatenate([s, sv], axis=0))
            for t in range(NT):
                order = list(range(nm))
                for j in reversed(range(nv)):
                    order.insert(1 + ((j * NT + t) * nm) // (nv * NT), nm + j)
                acc = lsums[sub][t]
                for b in order:
                    blk = p[b * 8:(b + 1) * 8, t * LANE:(t + 1) * LANE]
                    acc = blk if acc is None else acc + blk
                lsums[sub][t] = acc
            ps[(sub, c)] = p.astype(BF16)

        def pv(sub, c):
            vt = _unpk(vt_ref[c, pl.ds(h0, DH // 2), :])
            o = jnp.dot(vt, ps.pop((sub, c)), preferred_element_type=F32)
            accs[sub] = (z_ref[...] if c == 0 else accs[sub]) + o
            if c == NB - 1:
                l = jnp.sum(_cat(lsums[sub], 1), axis=0, keepdims=True)
                o = accs[sub] * (1.0 / l)
                ob = _pk(o.astype(BF16))
                for t in range(NT):
                    ot_ref[sub * NT + t, pl.ds(h0, DH // 2), :] = ob[:, t * LANE:(t + 1) * LANE]
                flags[0] = jnp.maximum(flags[0], _bad_flag(l, o))

        n = len(steps)
        for i in range(n + SKEW):
            if i < n:
                qk(*steps[i])
            if i >= SKEW:
                pv(*steps[i - SKEW])
        return flags[0]

    return lax.fori_loop(0, H, body, jnp.zeros((1, TQ), F32))


def _sliding_attention(k_ref, qt_ref, vt_ref, ot_ref, z_ref):
    NH, SKEW = 4, 2
    NW = WIN // LANE

    def body(it, bad):
        g = it >> 1
        g0 = pl.multiple_of(g * (LANE // 2), LANE // 2)
        r0 = (it & 1) * NH
        hbase = it * NH
        row = lax.broadcasted_iota(jnp.int32, (LANE, NH * LANE), 0)
        col = lax.broadcasted_iota(jnp.int32, (LANE, NH * LANE), 1) & (LANE - 1)
        steps = [(j, c) for j in range(NB) for c in range(max(0, j - NW), j + 1)]
        ws, accs, lsums, ps = {}, {}, {}, {}
        flags = [bad]

        def qk(j, c):
            first = c == max(0, j - NW)
            if first:
                qt = qt_ref[j, pl.ds(g0, LANE // 2), :]
                ws[j] = jnp.concatenate(
                    [_head_weights(qt, r0 + u) for u in range(NH)], axis=1)
            kc = _unpk(k_ref[g, pl.ds(c * (LANE // 2), LANE // 2), :])
            s = jnp.dot(kc, ws[j], preferred_element_type=F32)
            p = jnp.exp2(s)
            if c == j:
                p = jnp.where(row <= col, p, 0.0)
            elif c == j - NW:
                p = jnp.where(row > col, p, 0.0)
            part = jnp.sum(p.reshape(LANE // 8, 8, NH * LANE), axis=0)
            lsums[j] = part if first else lsums[j] + part
            ps[(j, c)] = p.astype(BF16)

        def pv(j, c):
            first = c == max(0, j - NW)
            p = ps.pop((j, c))
            os = []
            for u in range(NH):
                h0 = pl.multiple_of((hbase + u) * (DH // 2), DH // 2)
                vt = _unpk(vt_ref[c, pl.ds(h0, DH // 2), :])
                os.append(jnp.dot(vt, p[:, u * LANE:(u + 1) * LANE],
                                  preferred_element_type=F32))
            o = jnp.concatenate(os, axis=1)
            accs[j] = (z_ref[...] if first else accs[j]) + o
            if c == j:
                l = jnp.sum(lsums.pop(j), axis=0, keepdims=True)
                o = accs.pop(j) * (1.0 / l)
                ob = _pk(o.astype(BF16))
                for u in range(NH):
                    h0 = pl.multiple_of((hbase + u) * (DH // 2), DH // 2)
                    ot_ref[j, pl.ds(h0, DH // 2), :] = ob[:, u * LANE:(u + 1) * LANE]
                flags[0] = jnp.maximum(flags[0], _bad_flag(l, o))

        n = len(steps)
        for i in range(n + SKEW):
            if i < n:
                qk(*steps[i])
            if i >= SKEW:
                pv(*steps[i - SKEW])
        return flags[0]

    return lax.fori_loop(0, H // NH, body, jnp.zeros((1, NH * LANE), F32))


def _safe_attention(k_ref, qt_ref, vt_ref, ot_ref, sliding):
    NKB = (WIN // LANE + 1) if sliding else NB
    NK = NKB * LANE

    def body(it, carry):
        h = it >> 4
        j = it & (NB - 1)
        g = h >> 3
        g0 = pl.multiple_of(g * (LANE // 2), LANE // 2)
        h0 = pl.multiple_of(h * (DH // 2), DH // 2)
        cb = jnp.maximum(j - WIN // LANE, 0) if sliding else 0
        k0 = cb * LANE
        k0h = pl.multiple_of(cb * (LANE // 2), LANE // 2) if sliding else 0
        w = _head_weights(qt_ref[j, pl.ds(g0, LANE // 2), :], h & (GROUP - 1))
        kc = _unpk(k_ref[g, pl.ds(k0h, NK // 2), :])
        s = jnp.dot(kc, w, preferred_element_type=F32)
        if sliding:
            kpos = k0 + lax.broadcasted_iota(jnp.int32, s.shape, 0)
            qpos = j * LANE + lax.broadcasted_iota(jnp.int32, s.shape, 1)
            d = qpos - kpos
            s = jnp.where(jnp.logical_and(d >= 0, d < WIN), s, -1e9)
        m = jnp.max(s, axis=0, keepdims=True)
        p = jnp.exp2(s - m)
        l = jnp.sum(p, axis=0, keepdims=True)
        p = (p * (1.0 / l)).astype(BF16)
        vt = _unpk(_cat([vt_ref[cb + i, pl.ds(h0, DH // 2), :] for i in range(NKB)], 1))
        o = jnp.dot(vt, p, preferred_element_type=F32)
        ot_ref[j, pl.ds(h0, DH // 2), :] = _pk(o.astype(BF16))
        return carry

    lax.fori_loop(0, H * NB, body, 0)


def _attention(k_ref, qt_ref, vt_ref, ot_ref, kb_ref, z_ref, sliding):
    if sliding:
        bad = _sliding_attention(k_ref, qt_ref, vt_ref, ot_ref, z_ref)
    else:
        bad = _full_attention(k_ref, qt_ref, vt_ref, ot_ref, kb_ref, z_ref)

    @pl.when(jnp.max(bad) > 0.0)
    def _():
        _safe_attention(k_ref, qt_ref, vt_ref, ot_ref, sliding)


def _layernorm(x):
    m = jnp.mean(x, axis=-1, keepdims=True)
    xc = x - m
    v = jnp.mean(xc * xc, axis=-1, keepdims=True)
    return (xc * lax.rsqrt(v + LN_EPS)).astype(BF16)


def _project_k(xn, i, wk, k_ref):
    k = _pk(jnp.dot(xn, wk, preferred_element_type=F32).astype(BF16))
    for g in range(NG):
        k_ref[g, pl.ds(_mo(i * (TM // 2), TM // 2), TM // 2), :] = k[:, g * LANE:(g + 1) * LANE]


def _project_qv(xn, i, wt, qt_ref, vt_ref):
    qv = lax.dot_general(wt, xn, (((1,), (1,)), ((), ())),
                         preferred_element_type=F32)
    qt = _pk((qv[:D] * QSCALE).astype(BF16))
    vt = _pk(qv[D:].astype(BF16))
    for t in range(TM // LANE):
        j = i * (TM // LANE) + t
        qt_ref[j] = qt[:, t * LANE:(t + 1) * LANE]
        vt_ref[j] = vt[:, t * LANE:(t + 1) * LANE]


def _project_out(i, ot_ref, wo):
    ot = _unpk(_cat([ot_ref[i * (TM // LANE) + t] for t in range(TM // LANE)], 1))
    return lax.dot_general(ot, wo, (((0,), (0,)), ((), ())),
                           preferred_element_type=F32)


def _kernel(x_hbm, wa_hbm, woa_hbm, wb_hbm, wob_hbm, o_hbm,
            xb_ref, w_ref, wo_ref, wt_ref,
            xres_ref, k_ref, qt_ref, vt_ref, ot_ref, kb_ref, z_ref, sems):
    nchunk = S // TM

    def rows(i):
        return pl.ds(_mo(i * TM, TM), TM)

    x_cp = [pltpu.make_async_copy(x_hbm.at[rows(i)], xb_ref.at[rows(i)], sems.at[i])
            for i in range(nchunk)]
    wa_cp = [pltpu.make_async_copy(wa_hbm.at[:, pl.ds(n * D, D)], w_ref.at[0, n],
                                   sems.at[nchunk + n]) for n in range(3)]
    wb_cp = [pltpu.make_async_copy(wb_hbm.at[:, pl.ds(n * D, D)], w_ref.at[1, n],
                                   sems.at[nchunk + 3 + n]) for n in range(3)]
    wo_cp = [pltpu.make_async_copy(src, wo_ref.at[n], sems.at[nchunk + 6 + n])
             for n, src in enumerate((woa_hbm, wob_hbm))]
    for cp in (x_cp[0], wa_cp[1], wa_cp[0], wa_cp[2], *x_cp[1:], *wb_cp, *wo_cp):
        cp.start()

    z_ref[...] = jnp.zeros(z_ref.shape, F32)

    def transpose_w(n):
        wt_ref[n, 0:D // 2, :] = _pk(w_ref[n, 0].T)
        wt_ref[n, D // 2:D, :] = _pk(w_ref[n, 2].T)

    def load_x(i):
        x = xb_ref[rows(i), :].astype(F32)
        xres_ref[rows(i), :] = x
        return _layernorm(x)

    x_cp[0].wait()
    xn0 = load_x(0)
    wa_cp[1].wait()
    _project_k(xn0, 0, w_ref[0, 1], k_ref)
    wa_cp[0].wait()
    wa_cp[2].wait()
    x_cp[1].wait()
    transpose_w(0)
    xn1 = load_x(1)
    _project_k(xn1, 1, w_ref[0, 1], k_ref)
    _project_qv(xn0, 0, _unpk(wt_ref[0]), qt_ref, vt_ref)
    for cp in (*x_cp[2:], *wb_cp, *wo_cp):
        cp.wait()
    _project_qv(xn1, 1, _unpk(wt_ref[0]), qt_ref, vt_ref)
    transpose_w(1)
    for i in range(2, nchunk):
        xn = load_x(i)
        _project_k(xn, i, w_ref[0, 1], k_ref)
        _project_qv(xn, i, _unpk(wt_ref[0]), qt_ref, vt_ref)

    def layer(t, carry):
        cur = t & 1

        @pl.when(cur == 0)
        def _():
            _attention(k_ref, qt_ref, vt_ref, ot_ref, kb_ref, z_ref, sliding=True)

        @pl.when(cur == 1)
        def _():
            _attention(k_ref, qt_ref, vt_ref, ot_ref, kb_ref, z_ref, sliding=False)

        @pl.when(t < 3)
        def _():
            nxt = 1 - cur

            def resid(i):
                x = xres_ref[rows(i), :] + _project_out(i, ot_ref, wo_ref[cur])
                xres_ref[rows(i), :] = x
                return _layernorm(x)

            def half(it, c):
                a, b = 2 * it, 2 * it + 1
                xa = resid(a)
                xb = resid(b)
                _project_k(xa, a, w_ref[nxt, 1], k_ref)
                _project_k(xb, b, w_ref[nxt, 1], k_ref)
                _project_qv(xa, a, _unpk(wt_ref[nxt]), qt_ref, vt_ref)
                _project_qv(xb, b, _unpk(wt_ref[nxt]), qt_ref, vt_ref)
                _prep_kb(0, k_ref, kb_ref, it * (NB // 2), NB // 2)
                return c

            lax.fori_loop(0, nchunk // 2, half, 0)
        return carry

    lax.fori_loop(0, 4, layer, 0)

    def o_cp(i):
        return pltpu.make_async_copy(xb_ref.at[rows(i)], o_hbm.at[rows(i)], sems.at[i])

    def last(it, c):
        for i in (2 * it, 2 * it + 1):
            x = xres_ref[rows(i), :] + _project_out(i, ot_ref, wo_ref[1])
            xb_ref[rows(i), :] = x.astype(BF16)
            o_cp(i).start()
        return c

    lax.fori_loop(0, nchunk // 2, last, 0)
    for i in range(nchunk):
        o_cp(i).wait()


@jax.jit
def pallas_interleave_layers__sliding_block__mha_block__prompt_kernel(
    A_x: jax.Array,
    A_wqkv: jax.Array,
    A_wo: jax.Array,
    B_x: jax.Array,
    B_wqkv: jax.Array,
    B_wo: jax.Array,
):
    del B_x
    x = A_x.reshape(S, D)
    any_spec = pl.BlockSpec(memory_space=pl.ANY)
    out = pl.pallas_call(
        _kernel,
        out_shape=jax.ShapeDtypeStruct((S, D), A_x.dtype),
        in_specs=[any_spec] * 5,
        out_specs=any_spec,
        scratch_shapes=[
            pltpu.VMEM((S, D), BF16),
            pltpu.VMEM((2, 3, D, D), BF16),
            pltpu.VMEM((2, D, D), BF16),
            pltpu.VMEM((2, D, D), U32),
            pltpu.VMEM((S, D), F32),
            pltpu.VMEM((NG, S // 2, LANE), U32),
            pltpu.VMEM((NB, D // 2, LANE), U32),
            pltpu.VMEM((NB, D // 2, LANE), U32),
            pltpu.VMEM((NB, D // 2, LANE), U32),
            pltpu.VMEM((DH, NB * RV // 2, LANE), U32),
            pltpu.VMEM((DH, 4 * LANE), F32),
            pltpu.SemaphoreType.DMA((S // TM + 8,)),
        ],
        compiler_params=pltpu.CompilerParams(vmem_limit_bytes=100 * 1024 * 1024),
    )(x, A_wqkv, A_wo, B_wqkv, B_wo)
    return out.reshape(A_x.shape)
```

```python
import math

import jax
import jax.numpy as jnp
from jax import lax
import jax.experimental.pallas as pl
import jax.experimental.pallas.tpu as pltpu

S = 2048
D = 512
H = 32
DH = D // H
WIN = 256
LANE = 128
GROUP = LANE // DH
NG = D // LANE
NB = S // LANE
QSCALE = (DH ** -0.5) * math.log2(math.e)
LN_EPS = 1e-5
L_LO = 2.0 ** -40
L_HI = 2.0 ** 40
V_HI = 2.0 ** 60
NEG = -1e30

TM = 512
TO = 128
GK = 32
RV = 16
LAG_A = 2
HPI = 2
SKEW = 2
VPOS = (0, 0, 3, 5, 7, 9, 11, 13)
F32 = jnp.float32
BF16 = jnp.bfloat16
U32 = jnp.uint32


def _cat(xs, axis):
    return xs[0] if len(xs) == 1 else jnp.concatenate(xs, axis=axis)


def _pk(x):
    return pltpu.bitcast(x, U32)


def _unpk(x):
    return pltpu.bitcast(x, BF16)


def _head_weights(q32, r):
    rows = lax.broadcasted_iota(jnp.int32, q32.shape, 0) >> 3
    return pltpu.bitcast(jnp.where(rows == r, q32, jnp.uint32(0)), BF16)


def _normalize(acc, lsum, bad):
    l = jnp.sum(lsum, axis=0, keepdims=True)
    r = pl.reciprocal(l, approx=True)
    r = r * (2.0 - l * r)
    ok = jnp.logical_and(l >= L_LO, l <= L_HI)
    return acc * r, jnp.where(ok, bad, 1.0)


def _mo(x, m):
    return x if isinstance(x, int) else pl.multiple_of(x, m)


def _prep_kb(h, k_ref, kb_ref, c0=0, nc=NB):
    kk = _cat([k_ref[h >> 3, pl.ds(_mo((c0 + c) * (LANE // 2) + (LANE - RV) // 2, 8), RV // 2), :]
               for c in range(nc)], 0)
    if not (isinstance(h, int) and h % GROUP == 0):
        kk = pltpu.roll(kk, (LANE - (h & (GROUP - 1)) * DH) & (LANE - 1), 1)
    for d in range(DH):
        kb_ref[d, pl.ds(_mo(c0 * (RV // 2), 8), nc * (RV // 2)), :] = (
            jnp.broadcast_to(kk[:, d:d + 1], kk.shape))


def _init_carry(pc_ref, ac_ref):
    pc_ref[...] = jnp.zeros(pc_ref.shape, U32)
    ac_ref[...] = jnp.ones(ac_ref.shape, F32)


def _full_attention(k_ref, qt_ref, vt_ref, ot_ref, kb_ref, z_ref, pc_ref, ac_ref):
    NT = 4
    TQ = NT * LANE
    NSUB = NB // NT
    nm = (LANE - RV) // 8
    steps = [(sub, c) for sub in range(NSUB) for c in range(NB)]
    n = len(steps)
    tail = steps[n - SKEW:]

    def finish(h0, sub, acc, lsum, bad):
        o, bad = _normalize(acc, lsum, bad)
        for t in range(NT):
            ot_ref[sub * NT + t, pl.ds(h0, DH // 2), :] = _pk(
                o[:, t * LANE:(t + 1) * LANE].astype(BF16))
        return bad

    def tail_step(i, h0, acc):
        vt = _unpk(vt_ref[tail[i][1], pl.ds(h0, DH // 2), :])
        if i == 0:
            acc = ac_ref[0:DH, :]
        return acc + jnp.dot(vt, _unpk(pc_ref[i]), preferred_element_type=F32)

    def body(it, bad):
        g = (it * HPI) >> 3
        g0 = pl.multiple_of(g * (LANE // 2), LANE // 2)
        hp0 = pl.multiple_of(jnp.maximum(it * HPI - 1, 0) * (DH // 2), DH // 2)
        ws, qbs, kbs, accs, lsums, ps = {}, {}, {}, {}, {}, {}
        flags = [bad]

        def row0(u):
            return pl.multiple_of((it * HPI + u) * (DH // 2), DH // 2)

        def qk(u, sub, c):
            h = it * HPI + u
            if c == 0:
                blks = range(sub * NT, (sub + 1) * NT)
                ws[0] = _head_weights(
                    _cat([qt_ref[j, pl.ds(g0, LANE // 2), :] for j in blks], 1),
                    h & (GROUP - 1))
                qh = _unpk(_cat([qt_ref[j, pl.ds(row0(u), DH // 2), :] for j in blks], 1))
                qh = qh.astype(F32)
                qbs[0] = [jnp.broadcast_to(qh[d:d + 1, :], (8, TQ)) for d in range(DH)]
                lsums[(u, sub)] = [None] * NT
            if sub == 0:
                kbs[c] = [_unpk(kb_ref[u, d, pl.ds(c * (RV // 2), RV // 2), :]).astype(F32)
                          for d in range(DH)]
                if c == NB - 1:
                    _prep_kb(jnp.minimum(h + HPI, H - 1), k_ref, kb_ref.at[u])
            kc = _unpk(k_ref[g, pl.ds(c * (LANE // 2), (LANE - RV) // 2), :])
            pm = jnp.exp2(jnp.dot(kc, ws[0], preferred_element_type=F32))
            sv = None
            for d in range(DH):
                t = _cat([kbs[c][d]] * NT, 1) * _cat([qbs[0][d]] * (RV // 8), 0)
                sv = t if sv is None else sv + t
            pvp = jnp.exp2(sv)
            for t in range(NT):
                acc = lsums[(u, sub)][t]
                for b in range(nm + 1):
                    blks = [pvp[j * 8:(j + 1) * 8, t * LANE:(t + 1) * LANE]
                            for j in range(RV // 8) if VPOS[j * NT + t] == b]
                    if b < nm:
                        blks.append(pm[b * 8:(b + 1) * 8, t * LANE:(t + 1) * LANE])
                    for blk in blks:
                        acc = blk if acc is None else acc + blk
                lsums[(u, sub)][t] = acc
            ps[(u, sub, c)] = jnp.concatenate([pm, pvp], axis=0).astype(BF16)

        def pv(u, sub, c):
            vt = _unpk(vt_ref[c, pl.ds(row0(u), DH // 2), :])
            o = jnp.dot(vt, ps.pop((u, sub, c)), preferred_element_type=F32)
            accs[0] = (z_ref[...] if c == 0 else accs[0]) + o
            if c == NB - 1:
                flags[0] = finish(row0(u), sub, accs[0], _cat(lsums[(u, sub)], 1), flags[0])

        allsteps = [(u, sub, c) for u in range(HPI) for (sub, c) in steps]
        pacc = None
        for i, st in enumerate(allsteps):
            qk(*st)
            if i >= SKEW:
                pv(*allsteps[i - SKEW])
            else:
                pacc = tail_step(i, hp0, pacc)
                if i == SKEW - 1:
                    flags[0] = finish(hp0, NSUB - 1, pacc, ac_ref[DH:DH + 8, :], flags[0])
        never = pltpu.bitcast(z_ref[0:RV // 2, :], U32) != 0
        nmh = (LANE - RV) // 2
        for i in range(SKEW):
            pp = _pk(ps.pop((HPI - 1,) + tail[i]))
            pc_ref[i] = jnp.concatenate(
                [pp[:nmh], jnp.where(never, pp[0:RV // 2], pp[nmh:])], axis=0)
        ac_ref[0:DH, :] = accs[0]
        ac_ref[DH:DH + 8, :] = _cat(lsums[(HPI - 1, NSUB - 1)], 1)
        return flags[0]

    bad = lax.fori_loop(0, H // HPI, body, jnp.zeros((1, TQ), F32))
    pacc = None
    for i in range(SKEW):
        pacc = tail_step(i, (H - 1) * (DH // 2), pacc)
    return finish((H - 1) * (DH // 2), NSUB - 1, pacc, ac_ref[DH:DH + 8, :], bad)


def _init_bias(bias_ref):
    row = lax.broadcasted_iota(jnp.int32, (LANE, LANE), 0)
    col = lax.broadcasted_iota(jnp.int32, (LANE, LANE), 1)
    bias_ref[0] = jnp.where(row <= col, 0.0, NEG)
    bias_ref[1] = jnp.where(jnp.logical_or(col < row, col >= row + GK), 0.0, NEG)


def _sliding_attention(k_ref, qt_ref, vt_ref, ot_ref, z_ref, pc_ref, ac_ref, bias_ref):
    NH = 4
    HL = LANE // 2
    W = NH * LANE
    NC = LANE // GK - 1
    GH = GK // 2

    def pv_tile(b, hbase, tiles, acc):
        os = [jnp.dot(_unpk(vt_ref[b, pl.ds(_mo((hbase + u) * (DH // 2), DH // 2), DH // 2), :]),
                      tiles[u], preferred_element_type=F32) for u in range(NH)]
        return (z_ref[...] if acc is None else acc) + jnp.concatenate(os, axis=1)

    def finish(j, hbase, acc, lsum, bad):
        o, bad = _normalize(acc, lsum, bad)
        for u in range(NH):
            h0 = _mo((hbase + u) * (DH // 2), DH // 2)
            ot_ref[j, pl.ds(h0, DH // 2), :] = _pk(
                o[:, u * LANE:(u + 1) * LANE].astype(BF16))
        return bad

    def tail_step(i, hbase, acc):
        tiles = [_unpk(pc_ref[i, :, u * LANE:(u + 1) * LANE]) for u in range(NH)]
        return pv_tile(NB - 3 + i, hbase, tiles, acc)

    def body(it, bad):
        g = it >> 1
        g0 = pl.multiple_of(g * HL, HL)
        par = it & 1
        hbase = it * NH
        own_rows = (lax.broadcasted_iota(jnp.int32, (HL, LANE), 0) >> 5) == par
        lane_w = lax.broadcasted_iota(jnp.int32, (HL, LANE), 1)
        lane_p = lax.broadcasted_iota(jnp.int32, (GK, LANE), 1)
        own_lanes = (lax.broadcasted_iota(jnp.int32, (GH, LANE), 1) >> 6) == par
        zero32 = jnp.uint32(0)
        flags = [bad]
        lsums, accs, groups = {}, {}, {}

        def spread(m):
            z = jnp.zeros((8, LANE), U32)
            tiles = [_cat([m[rb * 8:(rb + 1) * 8] if rb % NH == u else z
                           for rb in range(2 * NH)], 0) for u in range(NH)]
            return _unpk(_cat(tiles, 1))

        def krows(r0, m):
            return k_ref[g, pl.ds(r0 // 2, m // 2), :]

        def bias(n, r0):
            return _cat([bias_ref[n, r0:r0 + GK, :]] * NH, 1)

        def probs(j, kc, w, biases):
            s = jnp.dot(_unpk(kc), w, preferred_element_type=F32)
            s = _cat([s[n * GK:(n + 1) * GK] if bs is None
                      else s[n * GK:(n + 1) * GK] + bias(*bs)
                      for n, bs in enumerate(biases)], 0)
            p = jnp.exp2(s)
            part = jnp.sum(p.reshape(p.shape[0] // 8, 8, W), axis=0)
            lsums[j] = part if j not in lsums else lsums[j] + part
            return p

        def passes(j):
            qt = qt_ref[j, pl.ds(g0, HL), :]
            w = spread(jnp.where(own_rows, qt, zero32))
            k0 = j * LANE

            def shared(m0, m1):
                def run():
                    biases = [(1, NC * GK) if m == -5 else (0, m * GK) if m >= 0 else None
                              for m in range(m0, m1)]
                    p = probs(j, krows(k0 + m0 * GK, (m1 - m0) * GK), w, biases)
                    for m in range(m0, m1):
                        groups[(j, m)] = p[(m - m0) * GK:(m - m0 + 1) * GK]
                return run

            if j < 2:
                return [shared(m, m + 2) for m in range(-4 * j, 4, 2)]
            qmix = jnp.where(own_rows, qt,
                             jnp.concatenate([qt[HL // 2:], qt[:HL // 2]], axis=0))

            def combined(i):
                def run():
                    split = (i + 1) * GK
                    wc = spread(jnp.where(own_rows == (lane_w < split), qmix, zero32))
                    kc = jnp.where(own_lanes, krows(k0 - WIN + i * GK, GK),
                                   pltpu.roll(krows(k0 + split, GK), HL, 1))
                    p = probs(j, kc, wc, [(1, i * GK)])
                    low = _cat([lane_p < split] * NH, 1)
                    groups[(j, i - 8)] = jnp.where(low, p, 0.0)
                    groups[(j, i + 1)] = jnp.where(low, 0.0, p)
                return run

            out = []
            for i in range(NC):
                sh, cb = shared(-5 + 2 * i, -3 + 2 * i), combined(i)
                out.append(lambda sh=sh, cb=cb: (sh(), cb()))
            return out

        def tile(j, b):
            p = _cat([groups.pop((j, m)) for m in range(4 * (b - j), 4 * (b - j) + 4)], 0)
            return [p[:, u * LANE:(u + 1) * LANE].astype(BF16) for u in range(NH)]

        def pv(j, b):
            accs[j] = pv_tile(b, hbase, tile(j, b), accs.get(j))
            if b == j:
                flags[0] = finish(j, hbase, accs.pop(j), lsums.pop(j), flags[0])

        hprev = jnp.maximum(hbase - NH, 0)

        def tail(i):
            accs[-1] = tail_step(i, hprev, accs.get(-1))
            if i == 2:
                flags[0] = finish(NB - 1, hprev, accs.pop(-1), ac_ref[DH:DH + 8, :], flags[0])

        pending = [(0, lambda i=i: tail(i)) for i in range(3)]
        slot = 0
        for j in range(NB):
            for run in passes(j):
                run()
                if pending and pending[0][0] <= slot:
                    pending.pop(0)[1]()
                slot += 1
            if j < NB - 1:
                pending += [(slot + LAG_A, lambda j=j, b=b: pv(j, b))
                            for b in range(max(j - 2, 0), j + 1)]
        for _, job in pending:
            job()
        for i in range(3):
            for u, t in enumerate(tile(NB - 1, NB - 3 + i)):
                pc_ref[i, :, u * LANE:(u + 1) * LANE] = _pk(t)
        ac_ref[DH:DH + 8, :] = lsums.pop(NB - 1)
        return flags[0]

    bad = lax.fori_loop(0, H // NH, body, jnp.zeros((1, W), F32))
    pacc = None
    for i in range(3):
        pacc = tail_step(i, H - NH, pacc)
    return finish(NB - 1, H - NH, pacc, ac_ref[DH:DH + 8, :], bad)


def _safe_attention(k_ref, qt_ref, vt_ref, ot_ref, sliding):
    NKB = (WIN // LANE + 1) if sliding else NB
    NK = NKB * LANE

    def body(it, carry):
        h = it >> 4
        j = it & (NB - 1)
        g = h >> 3
        g0 = pl.multiple_of(g * (LANE // 2), LANE // 2)
        h0 = pl.multiple_of(h * (DH // 2), DH // 2)
        cb = jnp.maximum(j - WIN // LANE, 0) if sliding else 0
        k0h = _mo(cb * (LANE // 2), LANE // 2)
        w = _head_weights(qt_ref[j, pl.ds(g0, LANE // 2), :], h & (GROUP - 1))
        kc = _unpk(k_ref[g, pl.ds(k0h, NK // 2), :])
        s = jnp.dot(kc, w, preferred_element_type=F32)
        if sliding:
            kpos = cb * LANE + lax.broadcasted_iota(jnp.int32, s.shape, 0)
            qpos = j * LANE + lax.broadcasted_iota(jnp.int32, s.shape, 1)
            d = qpos - kpos
            s = jnp.where(jnp.logical_and(d >= 0, d < WIN), s, -1e9)
        m = jnp.max(s, axis=0, keepdims=True)
        p = jnp.exp2(s - m)
        l = jnp.sum(p, axis=0, keepdims=True)
        p = (p * (1.0 / l)).astype(BF16)
        vt = _unpk(_cat([vt_ref[cb + i, pl.ds(h0, DH // 2), :] for i in range(NKB)], 1))
        o = jnp.dot(vt, p, preferred_element_type=F32)
        ot_ref[j, pl.ds(h0, DH // 2), :] = _pk(o.astype(BF16))
        return carry

    lax.fori_loop(0, H * NB, body, 0)


def _attention(k_ref, qt_ref, vt_ref, ot_ref, kb_ref, z_ref, pc_ref, ac_ref, bias_ref,
               vflag_ref, sliding):
    if sliding:
        bad = _sliding_attention(k_ref, qt_ref, vt_ref, ot_ref, z_ref, pc_ref, ac_ref, bias_ref)
    else:
        bad = _full_attention(k_ref, qt_ref, vt_ref, ot_ref, kb_ref, z_ref, pc_ref, ac_ref)

    bad = jnp.maximum(bad, jnp.max(vflag_ref[...].reshape(S // TM * 8, TM), axis=0, keepdims=True))

    @pl.when(jnp.max(bad) > 0.0)
    def _():
        _safe_attention(k_ref, qt_ref, vt_ref, ot_ref, sliding)


def _layernorm(x):
    m = jnp.mean(x, axis=-1, keepdims=True)
    xc = x - m
    v = jnp.mean(xc * xc, axis=-1, keepdims=True)
    return (xc * lax.rsqrt(v + LN_EPS)).astype(BF16)


def _project_k(xn, i, wk, k_ref, g0=0):
    k = jnp.dot(xn, wk, preferred_element_type=F32)
    for g in range(wk.shape[1] // LANE):
        k_ref[g0 + g, pl.ds(_mo(i * (TM // 2), TM // 2), TM // 2), :] = _pk(
            k[:, g * LANE:(g + 1) * LANE].astype(BF16))


def _project_qv(xn, i, wt, qt_ref, vt_ref, vflag_ref):
    qv = lax.dot_general(wt, xn, (((1,), (1,)), ((), ())),
                         preferred_element_type=F32)
    for t in range(TM // LANE):
        j = i * (TM // LANE) + t
        qt_ref[j] = _pk((qv[:D, t * LANE:(t + 1) * LANE] * QSCALE).astype(BF16))
        vt_ref[j] = _pk(qv[D:, t * LANE:(t + 1) * LANE].astype(BF16))
    big = jnp.where(jnp.abs(qv[D:]) < V_HI, 0.0, 1.0)
    vflag_ref[i] = jnp.max(big.reshape(D // 8, 8, TM), axis=0)


def _project_out(i, ot_ref, wo, tm=TM):
    ot = _unpk(_cat([ot_ref[i * (tm // LANE) + t] for t in range(tm // LANE)], 1))
    return lax.dot_general(ot, wo, (((0,), (0,)), ((), ())),
                           preferred_element_type=F32)


def _kernel(x_hbm, wa_hbm, woa_hbm, wb_hbm, wob_hbm, o_hbm,
            xb_ref, w_ref, wo_ref, wt_ref, xres_ref, xn_ref,
            k_ref, qt_ref, vt_ref, ot_ref, kb_ref, z_ref, pc_ref, ac_ref, bias_ref, vflag_ref, sems):
    nchunk = S // TM

    def rows(i):
        return pl.ds(_mo(i * TM, TM), TM)

    x_cp = [pltpu.make_async_copy(x_hbm.at[rows(i)], xb_ref.at[rows(i)], sems.at[i])
            for i in range(nchunk)]
    wa_cp = [pltpu.make_async_copy(wa_hbm.at[:, pl.ds(n * D, D)], w_ref.at[0, n],
                                   sems.at[nchunk + n]) for n in range(3)]
    wb_cp = [pltpu.make_async_copy(wb_hbm.at[:, pl.ds(n * D, D)], w_ref.at[1, n],
                                   sems.at[nchunk + 3 + n]) for n in range(3)]
    wo_cp = [pltpu.make_async_copy(src, wo_ref.at[n], sems.at[nchunk + 6 + n])
             for n, src in enumerate((woa_hbm, wob_hbm))]
    for cp in (x_cp[0], wa_cp[1], *x_cp[1:], wa_cp[0], wa_cp[2],
               wb_cp[0], wb_cp[2], wb_cp[1], *wo_cp):
        cp.start()

    z_ref[...] = jnp.zeros(z_ref.shape, F32)
    _init_bias(bias_ref)
    _init_carry(pc_ref, ac_ref)

    def normalize(i, x):
        xres_ref[rows(i), :] = x
        return _layernorm(x)

    def project_qv(i, xn, kind):
        _project_qv(xn, i, _unpk(wt_ref[kind]), qt_ref, vt_ref, vflag_ref)

    def stash(i):
        xn = normalize(i, xb_ref[rows(i), :].astype(F32))
        xn_ref[i] = _pk(xn)
        return xn

    def first_k(xn, i, half):
        _project_k(xn, i, w_ref[0, 1, :, half * (D // 2):(half + 1) * (D // 2)], k_ref,
                   half * (NG // 2))

    x_cp[0].wait()
    xn0 = stash(0)
    wa_cp[1].wait()
    first_k(xn0, 0, 0)
    x_cp[1].wait()
    first_k(xn0, 0, 1)
    xn1 = stash(1)
    first_k(xn1, 1, 0)
    x_cp[2].wait()
    x_cp[3].wait()
    first_k(xn1, 1, 1)
    xn2 = stash(2)
    _project_k(xn2, 2, w_ref[0, 1], k_ref)
    xn3 = stash(3)
    first_k(xn3, 3, 0)
    wa_cp[0].wait()
    wa_cp[2].wait()
    first_k(xn3, 3, 1)
    wt_ref[0, 0:D // 2, :] = _pk(w_ref[0, 0].T)
    wt_ref[0, D // 2:D, :] = _pk(w_ref[0, 2].T)

    def first_qv(it, c):
        n = 2 * it
        pltpu.make_async_copy(wb_hbm.at[:, pl.ds(pl.multiple_of(n * D, D), D)],
                              w_ref.at[1, n], sems.at[nchunk + 3 + n]).wait()
        for i in (2 * it, 2 * it + 1):
            project_qv(i, _unpk(xn_ref[i]), 0)
        wt_ref[1, pl.ds(pl.multiple_of(it * (D // 2), D // 2), D // 2), :] = _pk(w_ref[1, n].T)
        return c

    lax.fori_loop(0, 2, first_qv, 0)
    for cp in (wb_cp[1], *wo_cp):
        cp.wait()

    def layer(t, carry):
        cur = t & 1

        @pl.when(cur == 0)
        def _():
            _attention(k_ref, qt_ref, vt_ref, ot_ref, kb_ref, z_ref, pc_ref, ac_ref, bias_ref,
                       vflag_ref, sliding=True)

        @pl.when(cur == 1)
        def _():
            _attention(k_ref, qt_ref, vt_ref, ot_ref, kb_ref, z_ref, pc_ref, ac_ref, bias_ref,
                       vflag_ref, sliding=False)

        @pl.when(t < 3)
        def _():
            nxt = 1 - cur

            def resid(i):
                return normalize(
                    i, xres_ref[rows(i), :] + _project_out(i, ot_ref, wo_ref[cur]))

            def half(it, c):
                a, b = 2 * it, 2 * it + 1
                xa = resid(a)
                xb = resid(b)
                _project_k(xa, a, w_ref[nxt, 1], k_ref)
                _project_k(xb, b, w_ref[nxt, 1], k_ref)
                project_qv(a, xa, nxt)
                project_qv(b, xb, nxt)
                for u in range(HPI):
                    _prep_kb(u, k_ref, kb_ref.at[u], it * (NB // 2), NB // 2)
                _init_carry(pc_ref, ac_ref)
                return c

            lax.fori_loop(0, nchunk // 2, half, 0)
        return carry

    lax.fori_loop(0, 4, layer, 0)

    o_cp = [pltpu.make_async_copy(xb_ref.at[pl.ds(i * TO, TO)], o_hbm.at[pl.ds(i * TO, TO)],
                                  sems.at[i]) for i in range(S // TO)]
    for i in range(S // TO):
        x = xres_ref[pl.ds(i * TO, TO), :] + _project_out(i, ot_ref, wo_ref[1], TO)
        xb_ref[pl.ds(i * TO, TO), :] = x.astype(BF16)
        o_cp[i].start()
    for cp in o_cp:
        cp.wait()


@jax.jit
def pallas_interleave_layers__sliding_block__mha_block__prompt_kernel(
    A_x: jax.Array,
    A_wqkv: jax.Array,
    A_wo: jax.Array,
    B_x: jax.Array,
    B_wqkv: jax.Array,
    B_wo: jax.Array,
):
    del B_x
    x = A_x.reshape(S, D)
    any_spec = pl.BlockSpec(memory_space=pl.ANY)
    out = pl.pallas_call(
        _kernel,
        out_shape=jax.ShapeDtypeStruct((S, D), A_x.dtype),
        in_specs=[any_spec] * 5,
        out_specs=any_spec,
        scratch_shapes=[
            pltpu.VMEM((S, D), BF16),
            pltpu.VMEM((2, 3, D, D), BF16),
            pltpu.VMEM((2, D, D), BF16),
            pltpu.VMEM((2, D, D), U32),
            pltpu.VMEM((S, D), F32),
            pltpu.VMEM((S // TM, TM // 2, D), U32),
            pltpu.VMEM((NG, S // 2, LANE), U32),
            pltpu.VMEM((NB, D // 2, LANE), U32),
            pltpu.VMEM((NB, D // 2, LANE), U32),
            pltpu.VMEM((NB, D // 2, LANE), U32),
            pltpu.VMEM((HPI, DH, NB * RV // 2, LANE), U32),
            pltpu.VMEM((DH, 4 * LANE), F32),
            pltpu.VMEM((3, LANE // 2, 4 * LANE), U32),
            pltpu.VMEM((DH + 8, 4 * LANE), F32),
            pltpu.VMEM((2, LANE, LANE), F32),
            pltpu.VMEM((S // TM, 8, TM), F32),
            pltpu.SemaphoreType.DMA((max(S // TM + 8, S // TO),)),
        ],
        compiler_params=pltpu.CompilerParams(vmem_limit_bytes=100 * 1024 * 1024),
    )(x, A_wqkv, A_wo, B_wqkv, B_wo)
    return out.reshape(A_x.shape)
```

```python
import math

import jax
import jax.numpy as jnp
from jax import lax
import jax.experimental.pallas as pl
import jax.experimental.pallas.tpu as pltpu

S = 2048
D = 512
H = 32
DH = D // H
WIN = 256
LANE = 128
GROUP = LANE // DH
NG = D // LANE
NB = S // LANE
QSCALE = (DH ** -0.5) * math.log2(math.e)
LN_EPS = 1e-5
L_LO = 2.0 ** -60
L_HI = 2.0 ** 60
V_HI = 2.0 ** 60
NEG = -1e30

TM = 512
TR = 128
TO = 128
GK = 32
RV = 16
LAG_A = 2
HPI = 2
SKEW = 2
STAG = (11, 12, 13, 14)
VPOS = (0, 0, 3, 5, 7, 9, 11, 13)
XC = 9
XSTEPS = (25, 41, 57, 89, 105, 121)
XPOS = 12
VPOSX = (0, 0, 2, 4, 6, 8, 10, 11)
F32 = jnp.float32
BF16 = jnp.bfloat16
U32 = jnp.uint32


def _cat(xs, axis):
    return xs[0] if len(xs) == 1 else jnp.concatenate(xs, axis=axis)


def _pk(x):
    return pltpu.bitcast(x, U32)


def _unpk(x):
    return pltpu.bitcast(x, BF16)


def _head_weights(q32, r):
    rows = lax.broadcasted_iota(jnp.int32, q32.shape, 0) >> 3
    return pltpu.bitcast(jnp.where(rows == r, q32, jnp.uint32(0)), BF16)


def _normalize(acc, lsum, bad):
    l = jnp.sum(lsum, axis=0, keepdims=True)
    r = pl.reciprocal(l, approx=True)
    r = r * (2.0 - l * r)
    ok = jnp.logical_and(l >= L_LO, l <= L_HI)
    return acc * r, jnp.where(ok, bad, 1.0)


def _mo(x, m):
    return x if isinstance(x, int) else pl.multiple_of(x, m)


def _prep_kb(h, k_ref, kb_ref, half=None):
    rel = [(XC % 8) * (LANE // 2) + (LANE - 2 * RV) // 2]
    rel += [c * (LANE // 2) + (LANE - RV) // 2 for c in range(NB // 2)]
    if half is None:
        rows, slot0 = (rel + [S // 4 + r for r in rel])[1:], 1
    else:
        rows, slot0 = [half * (S // 4) + r for r in rel], half * len(rel)
    kk = _cat([k_ref[h >> 3, pl.ds(_mo(r, 8), RV // 2), :] for r in rows], 0)
    if not (isinstance(h, int) and h % GROUP == 0):
        kk = pltpu.roll(kk, (LANE - (h & (GROUP - 1)) * DH) & (LANE - 1), 1)
    for d in range(DH):
        kb_ref[d, pl.ds(_mo(slot0 * (RV // 2), 8), kk.shape[0]), :] = (
            jnp.broadcast_to(kk[:, d:d + 1], kk.shape))


def _init_carry(pc_ref, ac_ref):
    pc_ref[...] = jnp.zeros(pc_ref.shape, U32)
    ac_ref[...] = jnp.ones(ac_ref.shape, F32)


def _full_attention(k_ref, qt_ref, vt_ref, ot_ref, kb_ref, z_ref, pc_ref, ac_ref):
    NT = 4
    NSUB = NB // NT
    n = HPI * NSUB * NB

    def keys(i):
        blks = [((i - STAG[t]) // NB + 1) % (HPI * NSUB) for t in range(NT)]
        return [(blk // NSUB, (blk % NSUB) * NT + t) for t, blk in enumerate(blks)]

    assert all(u == 0 for u, _ in keys(n - SKEW)) and keys(n - SKEW) == keys(n - 1)
    xhost = {}
    for ix in XSTEPS:
        assert ix % NB == XC and ix < n - SKEW
        todo = list(range(2 * NT))
        for i in range(ix - 8, ix):
            m = next(m for m in todo if keys(i)[m % NT] == keys(ix)[m % NT])
            todo.remove(m)
            xhost[i] = (ix, m)

    def finish(h0, j, acc, lsum, bad):
        o, bad = _normalize(acc, lsum, bad)
        ot_ref[j, pl.ds(h0, DH // 2), :] = _pk(o.astype(BF16))
        return bad

    def tail_step(i, h0, acc):
        vt = _unpk(vt_ref[NB - SKEW + i, pl.ds(h0, DH // 2), :])
        if i == 0:
            acc = ac_ref[0:DH, :]
        return acc + jnp.dot(vt, _unpk(pc_ref[i]), preferred_element_type=F32)

    def tail_finish(h0, acc, bad):
        for t, (_, j) in enumerate(keys(n - 1)):
            lanes = slice(t * LANE, (t + 1) * LANE)
            bad = finish(h0, j, acc[:, lanes], ac_ref[DH:DH + 8, lanes], bad)
        return bad

    def body(it, bad):
        g = (it * HPI) >> 3
        g0 = pl.multiple_of(g * (LANE // 2), LANE // 2)
        hp0 = pl.multiple_of(jnp.maximum(it - 1, 0) * (HPI * DH // 2), DH // 2)
        ws, qbs, kbs, accs, lsums, ps, pvs = {}, {}, {}, {}, {}, {}, {}
        remaining = {(u, j): NB for u in range(HPI) for j in range(NB)}
        flags = [bad]

        def row0(u):
            return pl.multiple_of((it * HPI + u) * (DH // 2), DH // 2)

        def setup(js):
            for u, j in js:
                if (u, j) not in ws:
                    ws[(u, j)] = _head_weights(qt_ref[j, pl.ds(g0, LANE // 2), :],
                                               (it * HPI + u) & (GROUP - 1))
                    qh = _unpk(qt_ref[j, pl.ds(row0(u), DH // 2), :]).astype(F32)
                    qbs[(u, j)] = [jnp.broadcast_to(qh[d:d + 1, :], (8, LANE))
                                   for d in range(DH)]

        def vgroup(i, x):
            if (i, x) not in pvs:
                js = keys(i)
                setup(js)
                c = i % NB
                slot = (c // 8) * 9 + (0 if x else 1 + c % 8)
                for u in set(k[0] for k in js):
                    if (u, slot) not in kbs:
                        kbs[(u, slot)] = [
                            _unpk(kb_ref[u, d, pl.ds(slot * (RV // 2), RV // 2), :]).astype(F32)
                            for d in range(DH)]
                        if sum(k[0] == u for k in kbs) == NB + 1:
                            _prep_kb(jnp.minimum(it * HPI + u + HPI, H - 1), k_ref, kb_ref.at[u])
                sv = None
                for d in range(DH):
                    qb = _cat([qbs[key][d] for key in js], 1)
                    t = _cat([kbs[(u, slot)][d] for u, _ in js], 1) * _cat([qb] * (RV // 8), 0)
                    sv = t if sv is None else sv + t
                pvs[(i, x)] = jnp.exp2(sv)
            return pvs[(i, x)]

        def qk(i):
            c = i % NB
            js = keys(i)
            setup(js)
            ng = 2 if i in XSTEPS else 1
            nm = (LANE - ng * RV) // 8
            kc = _unpk(k_ref[g, pl.ds(c * (LANE // 2), nm * 4), :])
            pm = jnp.exp2(jnp.dot(kc, _cat([ws[key] for key in js], 1),
                                  preferred_element_type=F32))
            hosted = [((VPOS if ng == 1 else VPOSX)[m], i, 0, m) for m in range(2 * NT)]
            if i in xhost:
                hosted.append((XPOS, xhost[i][0], 1, xhost[i][1]))
            for t, key in enumerate(js):
                acc = lsums.get(key)
                for b in range(nm + 1):
                    blks = [vgroup(ii, x)[(m // NT) * 8:(m // NT + 1) * 8,
                                          t * LANE:(t + 1) * LANE]
                            for pos, ii, x, m in hosted if pos == b and m % NT == t]
                    if b < nm:
                        blks.append(pm[b * 8:(b + 1) * 8, t * LANE:(t + 1) * LANE])
                    for blk in blks:
                        acc = blk if acc is None else acc + blk
                lsums[key] = acc
            ps[i] = jnp.concatenate(
                [pm] + [vgroup(i, x) for x in reversed(range(ng))], axis=0)

        def pv(i):
            js = keys(i)
            p = ps.pop(i)
            for u in sorted(set(k[0] for k in js)):
                ts = [t for t in range(NT) if js[t][0] == u]
                vt = _unpk(vt_ref[i % NB, pl.ds(row0(u), DH // 2), :])
                acc = _cat([accs.get(js[t], None) if js[t] in accs else z_ref[:, 0:LANE]
                            for t in ts], 1)
                acc = acc + jnp.dot(
                    vt, p[:, ts[0] * LANE:(ts[-1] + 1) * LANE].astype(BF16),
                    preferred_element_type=F32)
                for m, t in enumerate(ts):
                    key = js[t]
                    accs[key] = acc[:, m * LANE:(m + 1) * LANE]
                    remaining[key] -= 1
                    if remaining[key] == 0:
                        flags[0] = finish(row0(u), key[1], accs.pop(key), lsums.pop(key),
                                          flags[0])

        pacc = None
        for i in range(n):
            qk(i)
            if i >= SKEW:
                pv(i - SKEW)
            else:
                pacc = tail_step(i, hp0, pacc)
                if i == SKEW - 1:
                    flags[0] = tail_finish(hp0, pacc, flags[0])
        never = pltpu.bitcast(z_ref[0:RV // 2, :], U32) != 0
        nmh = (LANE - RV) // 2
        for i in range(SKEW):
            pp = _pk(ps.pop(n - SKEW + i).astype(BF16))
            pc_ref[i] = jnp.concatenate(
                [pp[:nmh], jnp.where(never, pp[0:RV // 2], pp[nmh:])], axis=0)
        ac_ref[0:DH, :] = _cat([accs[key] for key in keys(n - 1)], 1)
        ac_ref[DH:DH + 8, :] = _cat([lsums[key] for key in keys(n - 1)], 1)
        return flags[0]

    bad = lax.fori_loop(0, H // HPI, body, jnp.zeros((1, LANE), F32))
    pacc = None
    for i in range(SKEW):
        pacc = tail_step(i, (H - HPI) * (DH // 2), pacc)
    bad = tail_finish((H - HPI) * (DH // 2), pacc, bad)
    return _cat([bad] * NT, 1)


def _init_bias(bias_ref):
    row = lax.broadcasted_iota(jnp.int32, (LANE, LANE), 0)
    col = lax.broadcasted_iota(jnp.int32, (LANE, LANE), 1)
    bias_ref[0] = jnp.where(row <= col, 0.0, NEG)
    bias_ref[1] = jnp.where(jnp.logical_or(col < row, col >= row + GK), 0.0, NEG)


def _sliding_attention(k_ref, qt_ref, vt_ref, ot_ref, z_ref, pc_ref, ac_ref, bias_ref):
    NH = 4
    HL = LANE // 2
    W = NH * LANE
    NC = LANE // GK - 1
    GH = GK // 2

    def pv_tile(b, hbase, tiles, acc):
        os = [jnp.dot(_unpk(vt_ref[b, pl.ds(_mo((hbase + u) * (DH // 2), DH // 2), DH // 2), :]),
                      tiles[u], preferred_element_type=F32) for u in range(NH)]
        return (z_ref[...] if acc is None else acc) + jnp.concatenate(os, axis=1)

    def finish(j, hbase, acc, lsum, bad):
        o, bad = _normalize(acc, lsum, bad)
        for u in range(NH):
            h0 = _mo((hbase + u) * (DH // 2), DH // 2)
            ot_ref[j, pl.ds(h0, DH // 2), :] = _pk(
                o[:, u * LANE:(u + 1) * LANE].astype(BF16))
        return bad

    def tail_step(i, hbase, acc):
        tiles = [_unpk(pc_ref[i, :, u * LANE:(u + 1) * LANE]) for u in range(NH)]
        return pv_tile(NB - 3 + i, hbase, tiles, acc)

    def body(it, bad):
        g = it >> 1
        g0 = pl.multiple_of(g * HL, HL)
        par = it & 1
        hbase = it * NH
        own_rows = (lax.broadcasted_iota(jnp.int32, (HL, LANE), 0) >> 5) == par
        lane_w = lax.broadcasted_iota(jnp.int32, (HL, LANE), 1)
        lane_p = lax.broadcasted_iota(jnp.int32, (GK, LANE), 1)
        own_lanes = (lax.broadcasted_iota(jnp.int32, (GH, LANE), 1) >> 6) == par
        zero32 = jnp.uint32(0)
        flags = [bad]
        lsums, accs, groups = {}, {}, {}

        def spread(m):
            z = jnp.zeros((8, LANE), U32)
            tiles = [_cat([m[rb * 8:(rb + 1) * 8] if rb % NH == u else z
                           for rb in range(2 * NH)], 0) for u in range(NH)]
            return _unpk(_cat(tiles, 1))

        def krows(r0, m):
            return k_ref[g, pl.ds(r0 // 2, m // 2), :]

        def bias(n, r0):
            return _cat([bias_ref[n, r0:r0 + GK, :]] * NH, 1)

        def probs(j, kc, w, biases):
            s = jnp.dot(_unpk(kc), w, preferred_element_type=F32)
            s = _cat([s[n * GK:(n + 1) * GK] if bs is None
                      else s[n * GK:(n + 1) * GK] + bias(*bs)
                      for n, bs in enumerate(biases)], 0)
            p = jnp.exp2(s)
            part = jnp.sum(p.reshape(p.shape[0] // 8, 8, W), axis=0)
            lsums[j] = part if j not in lsums else lsums[j] + part
            return p

        def passes(j):
            qt = qt_ref[j, pl.ds(g0, HL), :]
            w = spread(jnp.where(own_rows, qt, zero32))
            k0 = j * LANE

            def shared(m0, m1):
                def run():
                    biases = [(1, NC * GK) if m == -5 else (0, m * GK) if m >= 0 else None
                              for m in range(m0, m1)]
                    p = probs(j, krows(k0 + m0 * GK, (m1 - m0) * GK), w, biases)
                    for m in range(m0, m1):
                        groups[(j, m)] = p[(m - m0) * GK:(m - m0 + 1) * GK]
                return run

            if j < 2:
                return [shared(m, m + 2) for m in range(-4 * j, 4, 2)]
            qmix = jnp.where(own_rows, qt,
                             jnp.concatenate([qt[HL // 2:], qt[:HL // 2]], axis=0))

            def combined(i):
                def run():
                    split = (i + 1) * GK
                    wc = spread(jnp.where(own_rows == (lane_w < split), qmix, zero32))
                    kc = jnp.where(own_lanes, krows(k0 - WIN + i * GK, GK),
                                   pltpu.roll(krows(k0 + split, GK), HL, 1))
                    p = probs(j, kc, wc, [(1, i * GK)])
                    low = _cat([lane_p < split] * NH, 1)
                    groups[(j, i - 8)] = jnp.where(low, p, 0.0)
                    groups[(j, i + 1)] = jnp.where(low, 0.0, p)
                return run

            out = []
            for i in range(NC):
                sh, cb = shared(-5 + 2 * i, -3 + 2 * i), combined(i)
                out.append(lambda sh=sh, cb=cb: (sh(), cb()))
            return out

        def tile(j, b):
            p = _cat([groups.pop((j, m)) for m in range(4 * (b - j), 4 * (b - j) + 4)], 0)
            return [p[:, u * LANE:(u + 1) * LANE].astype(BF16) for u in range(NH)]

        def pv(j, b):
            accs[j] = pv_tile(b, hbase, tile(j, b), accs.get(j))
            if b == j:
                flags[0] = finish(j, hbase, accs.pop(j), lsums.pop(j), flags[0])

        hprev = jnp.maximum(hbase - NH, 0)

        def tail(i):
            accs[-1] = tail_step(i, hprev, accs.get(-1))
            if i == 2:
                flags[0] = finish(NB - 1, hprev, accs.pop(-1), ac_ref[DH:DH + 8, :], flags[0])

        pending = [(0, lambda i=i: tail(i)) for i in range(3)]
        slot = 0
        for j in range(NB):
            for run in passes(j):
                run()
                if pending and pending[0][0] <= slot:
                    pending.pop(0)[1]()
                slot += 1
            if j < NB - 1:
                pending += [(slot + LAG_A, lambda j=j, b=b: pv(j, b))
                            for b in range(max(j - 2, 0), j + 1)]
        for _, job in pending:
            job()
        for i in range(3):
            for u, t in enumerate(tile(NB - 1, NB - 3 + i)):
                pc_ref[i, :, u * LANE:(u + 1) * LANE] = _pk(t)
        ac_ref[DH:DH + 8, :] = lsums.pop(NB - 1)
        return flags[0]

    bad = lax.fori_loop(0, H // NH, body, jnp.zeros((1, W), F32))
    pacc = None
    for i in range(3):
        pacc = tail_step(i, H - NH, pacc)
    return finish(NB - 1, H - NH, pacc, ac_ref[DH:DH + 8, :], bad)


def _safe_attention(k_ref, qt_ref, vt_ref, ot_ref, sliding):
    NKB = (WIN // LANE + 1) if sliding else NB
    NK = NKB * LANE

    def body(it, carry):
        h = it >> 4
        j = it & (NB - 1)
        g = h >> 3
        g0 = pl.multiple_of(g * (LANE // 2), LANE // 2)
        h0 = pl.multiple_of(h * (DH // 2), DH // 2)
        cb = jnp.maximum(j - WIN // LANE, 0) if sliding else 0
        k0h = _mo(cb * (LANE // 2), LANE // 2)
        w = _head_weights(qt_ref[j, pl.ds(g0, LANE // 2), :], h & (GROUP - 1))
        kc = _unpk(k_ref[g, pl.ds(k0h, NK // 2), :])
        s = jnp.dot(kc, w, preferred_element_type=F32)
        if sliding:
            kpos = cb * LANE + lax.broadcasted_iota(jnp.int32, s.shape, 0)
            qpos = j * LANE + lax.broadcasted_iota(jnp.int32, s.shape, 1)
            d = qpos - kpos
            s = jnp.where(jnp.logical_and(d >= 0, d < WIN), s, -1e9)
        m = jnp.max(s, axis=0, keepdims=True)
        p = jnp.exp2(s - m)
        l = jnp.sum(p, axis=0, keepdims=True)
        p = (p * (1.0 / l)).astype(BF16)
        vt = _unpk(_cat([vt_ref[cb + i, pl.ds(h0, DH // 2), :] for i in range(NKB)], 1))
        o = jnp.dot(vt, p, preferred_element_type=F32)
        ot_ref[j, pl.ds(h0, DH // 2), :] = _pk(o.astype(BF16))
        return carry

    lax.fori_loop(0, H * NB, body, 0)


def _attention(k_ref, qt_ref, vt_ref, ot_ref, kb_ref, z_ref, pc_ref, ac_ref, bias_ref,
               vflag_ref, sliding):
    if sliding:
        bad = _sliding_attention(k_ref, qt_ref, vt_ref, ot_ref, z_ref, pc_ref, ac_ref, bias_ref)
    else:
        bad = _full_attention(k_ref, qt_ref, vt_ref, ot_ref, kb_ref, z_ref, pc_ref, ac_ref)

    bad = jnp.maximum(bad, jnp.max(vflag_ref[...].reshape(S // TM * 8, TM), axis=0, keepdims=True))

    @pl.when(jnp.max(bad) > 0.0)
    def _():
        _safe_attention(k_ref, qt_ref, vt_ref, ot_ref, sliding)


def _layernorm(x):
    m = jnp.mean(x, axis=-1, keepdims=True)
    xc = x - m
    v = jnp.mean(xc * xc, axis=-1, keepdims=True)
    return (xc * lax.rsqrt(v + LN_EPS)).astype(BF16)


def _project_k(xn, i, wk, k_ref, g0=0):
    k = jnp.dot(xn, wk, preferred_element_type=F32)
    for g in range(wk.shape[1] // LANE):
        k_ref[g0 + g, pl.ds(_mo(i * (TM // 2), TM // 2), TM // 2), :] = _pk(
            k[:, g * LANE:(g + 1) * LANE].astype(BF16))


def _project_qv(xn, i, wt, qt_ref, vt_ref, vflag_ref):
    qv = lax.dot_general(wt, xn, (((1,), (1,)), ((), ())),
                         preferred_element_type=F32)
    for t in range(TM // LANE):
        j = i * (TM // LANE) + t
        qt_ref[j] = _pk((qv[:D, t * LANE:(t + 1) * LANE] * QSCALE).astype(BF16))
        vt_ref[j] = _pk(qv[D:, t * LANE:(t + 1) * LANE].astype(BF16))
    big = jnp.where(jnp.abs(qv[D:]) < V_HI, 0.0, 1.0)
    vflag_ref[i] = jnp.max(big.reshape(D // 8, 8, TM), axis=0)


def _project_out(i, ot_ref, wo, tm=TM):
    ot = _unpk(_cat([ot_ref[i * (tm // LANE) + t] for t in range(tm // LANE)], 1))
    return lax.dot_general(ot, wo, (((0,), (0,)), ((), ())),
                           preferred_element_type=F32)


def _kernel(x_hbm, wa_hbm, woa_hbm, wb_hbm, wob_hbm, o_hbm,
            xb_ref, w_ref, wo_ref, wt_ref, xres_ref, xn_ref,
            k_ref, qt_ref, vt_ref, ot_ref, kb_ref, z_ref, pc_ref, ac_ref, bias_ref, vflag_ref, sems):
    nchunk = S // TM

    def rows(i):
        return pl.ds(_mo(i * TM, TM), TM)

    x_cp = [pltpu.make_async_copy(x_hbm.at[rows(i)], xb_ref.at[rows(i)], sems.at[i])
            for i in range(nchunk)]
    wa_cp = [pltpu.make_async_copy(wa_hbm.at[:, pl.ds(n * D, D)], w_ref.at[0, n],
                                   sems.at[nchunk + n]) for n in range(3)]
    wb_cp = [pltpu.make_async_copy(wb_hbm.at[:, pl.ds(n * D, D)], w_ref.at[1, n],
                                   sems.at[nchunk + 3 + n]) for n in range(3)]
    wo_cp = [pltpu.make_async_copy(src, wo_ref.at[n], sems.at[nchunk + 6 + n])
             for n, src in enumerate((woa_hbm, wob_hbm))]
    for cp in (x_cp[0], wa_cp[1], *x_cp[1:], wa_cp[0], wa_cp[2],
               wb_cp[0], wb_cp[2], wb_cp[1], *wo_cp):
        cp.start()

    z_ref[...] = jnp.zeros(z_ref.shape, F32)
    _init_bias(bias_ref)
    _init_carry(pc_ref, ac_ref)

    def normalize(i, x):
        xres_ref[rows(i), :] = x
        return _layernorm(x)

    def project_qv(i, xn, kind):
        _project_qv(xn, i, _unpk(wt_ref[kind]), qt_ref, vt_ref, vflag_ref)

    def stash(i):
        xn = normalize(i, xb_ref[rows(i), :].astype(F32))
        xn_ref[i] = _pk(xn)
        return xn

    def first_k(xn, i, half):
        _project_k(xn, i, w_ref[0, 1, :, half * (D // 2):(half + 1) * (D // 2)], k_ref,
                   half * (NG // 2))

    x_cp[0].wait()
    xn0 = stash(0)
    wa_cp[1].wait()
    first_k(xn0, 0, 0)
    x_cp[1].wait()
    first_k(xn0, 0, 1)
    xn1 = stash(1)
    first_k(xn1, 1, 0)
    x_cp[2].wait()
    x_cp[3].wait()
    first_k(xn1, 1, 1)
    xn2 = stash(2)
    _project_k(xn2, 2, w_ref[0, 1], k_ref)
    xn3 = stash(3)
    first_k(xn3, 3, 0)
    wa_cp[0].wait()
    wa_cp[2].wait()
    first_k(xn3, 3, 1)
    wt_ref[0, 0:D // 2, :] = _pk(w_ref[0, 0].T)
    wt_ref[0, D // 2:D, :] = _pk(w_ref[0, 2].T)

    def first_qv(it, c):
        n = 2 * it
        pltpu.make_async_copy(wb_hbm.at[:, pl.ds(pl.multiple_of(n * D, D), D)],
                              w_ref.at[1, n], sems.at[nchunk + 3 + n]).wait()
        for i in (2 * it, 2 * it + 1):
            project_qv(i, _unpk(xn_ref[i]), 0)
        wt_ref[1, pl.ds(pl.multiple_of(it * (D // 2), D // 2), D // 2), :] = _pk(w_ref[1, n].T)
        return c

    lax.fori_loop(0, 2, first_qv, 0)
    for cp in (wb_cp[1], *wo_cp):
        cp.wait()

    def layer(t, carry):
        cur = t & 1

        @pl.when(cur == 0)
        def _():
            _attention(k_ref, qt_ref, vt_ref, ot_ref, kb_ref, z_ref, pc_ref, ac_ref, bias_ref,
                       vflag_ref, sliding=True)

        @pl.when(cur == 1)
        def _():
            _attention(k_ref, qt_ref, vt_ref, ot_ref, kb_ref, z_ref, pc_ref, ac_ref, bias_ref,
                       vflag_ref, sliding=False)

        @pl.when(t < 3)
        def _():
            nxt = 1 - cur

            def resid(i):
                xns = []
                for m in range(TM // TR):
                    r = pl.ds(pl.multiple_of(i * TM + m * TR, TR), TR)
                    x = xres_ref[r, :] + _project_out(i * (TM // TR) + m, ot_ref, wo_ref[cur], TR)
                    xres_ref[r, :] = x
                    xns.append(_layernorm(x))
                return _cat(xns, 0)

            def half(it, c):
                a, b = 2 * it, 2 * it + 1
                xa = resid(a)
                xb = resid(b)
                _project_k(xa, a, w_ref[nxt, 1], k_ref)
                _project_k(xb, b, w_ref[nxt, 1], k_ref)
                project_qv(a, xa, nxt)
                project_qv(b, xb, nxt)
                for u in range(HPI):
                    _prep_kb(u, k_ref, kb_ref.at[u], it)
                _init_carry(pc_ref, ac_ref)
                return c

            lax.fori_loop(0, nchunk // 2, half, 0)
        return carry

    lax.fori_loop(0, 4, layer, 0)

    o_cp = [pltpu.make_async_copy(xb_ref.at[pl.ds(i * TO, TO)], o_hbm.at[pl.ds(i * TO, TO)],
                                  sems.at[i]) for i in range(S // TO)]
    for i in range(S // TO):
        x = xres_ref[pl.ds(i * TO, TO), :] + _project_out(i, ot_ref, wo_ref[1], TO)
        xb_ref[pl.ds(i * TO, TO), :] = x.astype(BF16)
        o_cp[i].start()
    for cp in o_cp:
        cp.wait()


@jax.jit
def pallas_interleave_layers__sliding_block__mha_block__prompt_kernel(
    A_x: jax.Array,
    A_wqkv: jax.Array,
    A_wo: jax.Array,
    B_x: jax.Array,
    B_wqkv: jax.Array,
    B_wo: jax.Array,
):
    del B_x
    x = A_x.reshape(S, D)
    any_spec = pl.BlockSpec(memory_space=pl.ANY)
    out = pl.pallas_call(
        _kernel,
        out_shape=jax.ShapeDtypeStruct((S, D), A_x.dtype),
        in_specs=[any_spec] * 5,
        out_specs=any_spec,
        scratch_shapes=[
            pltpu.VMEM((S, D), BF16),
            pltpu.VMEM((2, 3, D, D), BF16),
            pltpu.VMEM((2, D, D), BF16),
            pltpu.VMEM((2, D, D), U32),
            pltpu.VMEM((S, D), F32),
            pltpu.VMEM((S // TM, TM // 2, D), U32),
            pltpu.VMEM((NG, S // 2, LANE), U32),
            pltpu.VMEM((NB, D // 2, LANE), U32),
            pltpu.VMEM((NB, D // 2, LANE), U32),
            pltpu.VMEM((NB, D // 2, LANE), U32),
            pltpu.VMEM((HPI, DH, (NB + 2) * RV // 2, LANE), U32),
            pltpu.VMEM((DH, 4 * LANE), F32),
            pltpu.VMEM((3, LANE // 2, 4 * LANE), U32),
            pltpu.VMEM((DH + 8, 4 * LANE), F32),
            pltpu.VMEM((2, LANE, LANE), F32),
            pltpu.VMEM((S // TM, 8, TM), F32),
            pltpu.SemaphoreType.DMA((max(S // TM + 8, S // TO),)),
        ],
        compiler_params=pltpu.CompilerParams(vmem_limit_bytes=100 * 1024 * 1024),
    )(x, A_wqkv, A_wo, B_wqkv, B_wo)
    return out.reshape(A_x.shape)
```

```python
import math

import jax
import jax.numpy as jnp
from jax import lax
import jax.experimental.pallas as pl
import jax.experimental.pallas.tpu as pltpu

S = 2048
D = 512
H = 32
DH = D // H
WIN = 256
LANE = 128
GROUP = LANE // DH
NG = D // LANE
NB = S // LANE
QSCALE = (DH ** -0.5) * math.log2(math.e)
LN_EPS = 1e-5
L_LO = 2.0 ** -60
L_HI = 2.0 ** 60
V_HI = 2.0 ** 60
NEG = -1e30

TM = 512
TR = 128
GK = 16
LAG_A = 2
HPI = 2
PR = HPI * DH // 2
NP = GROUP // HPI
RV = 16
QA = 2
SKEW = 2
STAG = (11, 12, 13, 14)
XREL = (2, 5, 7)
XSTEPS = (18, 21, 23, 26, 34, 37, 39, 42, 50, 53, 55, 58, 74, 82, 85, 87, 90, 98, 101, 103, 106, 114)
KB_HALF = 12
BORDER = (0, 4, 1, 5, 2, 6, 3, 7)
UTIL_MIN = 188
COST_Q = 60
COST_K = 56
COST_F = 10
COST_X = 30
XLU_STEPS = 14
START_SLOTS = 400
F32 = jnp.float32
BF16 = jnp.bfloat16
U32 = jnp.uint32


def _cat(xs, axis):
    return xs[0] if len(xs) == 1 else jnp.concatenate(xs, axis=axis)


def _pk(x):
    return pltpu.bitcast(x, U32)


def _unpk(x):
    return pltpu.bitcast(x, BF16)


def _swap8(x):
    y = x.reshape(x.shape[0] // 16, 2, 8, x.shape[1])
    return jnp.concatenate([y[:, 1:2], y[:, 0:1]], axis=1).reshape(x.shape)


def _hrows(j, u):
    return pl.ds(_mo((j * HPI + u) * (DH // 2), DH // 2), DH // 2)


def _head_weights(q32, r):
    rows = lax.broadcasted_iota(jnp.int32, q32.shape, 0) >> 3
    return pltpu.bitcast(jnp.where(rows == r, q32, jnp.uint32(0)), BF16)


def _normalize(acc, lsum, bad):
    l = jnp.sum(lsum, axis=0, keepdims=True)
    r = pl.reciprocal(l, approx=True)
    r = r * (2.0 - l * r)
    ok = jnp.logical_and(l >= L_LO, l <= L_HI)
    return acc * r, jnp.where(ok, bad, 1.0)


def _mo(x, m):
    return x if isinstance(x, int) else pl.multiple_of(x, m)


def _kb_slot(c, x):
    return (c // 8) * KB_HALF + (NB // 2 + XREL.index(c % 8) if x else c % 8)


def _prep_kb(pair, u, k_ref, kb_ref, half=None):
    if half is None:
        grps = [(c, 0) for c in range(NB)] + sorted({(i % NB, 1) for i in XSTEPS})
        half = 0
    else:
        grps = [(c, 0) for c in range(NB // 2)] + [(c, 1) for c in XREL]
    kk = _cat([k_ref[pair, pl.ds(_mo(half * (S // 4) + c * (LANE // 2) + x * (RV // 2), 8),
                                 RV // 2), :] for c, x in grps], 0)
    for d in range(DH):
        b = jnp.broadcast_to(kk[:, u * DH + d:u * DH + d + 1], kk.shape)
        for n, (c, x) in enumerate(grps):
            r0 = _mo((half * KB_HALF + _kb_slot(c, x)) * (RV // 2), 8)
            kb_ref[u, d, pl.ds(r0, RV // 2), :] = b[n * (RV // 2):(n + 1) * (RV // 2)]


def _plan_vpu(n, nt, keys):
    cost = 2 * DH + 1
    ngs = [2 if i in XSTEPS else 1 for i in range(n)]
    other, seen = [], set()
    for i in range(n):
        load = 2 * nt * (LANE - ngs[i] * RV) // 8 + 10
        new = {("q",) + k for k in keys(i)}
        load += COST_Q * len(new - seen)
        kbn = {("k", u, _kb_slot(i % NB, x)) for u, _ in keys(i) for x in range(ngs[i])}
        load += COST_K * len(kbn - seen)
        seen |= new | kbn
        if i > SKEW:
            load += COST_F * sum(a != b for a, b in zip(keys(i - SKEW - 1), keys(i - SKEW)))
        if i >= n - XLU_STEPS:
            load += COST_X
        other.append(load)

    def attempt(util):
        pool, frac, plan, ok = [], 0.0, {}, True
        for i in reversed(range(n)):
            pool += [(i, x, m) for x in range(ngs[i]) for m in BORDER]
            cap = util * 4 * (LANE + 16 - ngs[i] * RV) - other[i] + frac
            if i == 0:
                cap += START_SLOTS
            k = max(int(cap // cost), 0)
            frac = cap - k * cost
            must = [blk for blk in pool
                    if i == 0 or keys(i - 1)[blk[2] % nt] != keys(blk[0])[blk[2] % nt]]
            ok = ok and len(must) <= k + 1
            rest = [blk for blk in pool if blk not in must]
            rest.sort(key=lambda blk: blk[:2] != (i, 0))
            take = must + rest[:max(k - len(must), 0)]
            pool = [blk for blk in pool if blk not in take]
            plan[i] = sorted(take, key=lambda blk: (blk[0], blk[1], BORDER.index(blk[2])))
        return ok, plan

    util = next(v / 200 for v in range(UTIL_MIN, 240) if attempt(v / 200)[0])
    plan = attempt(util)[1]
    out = {}
    for i, blks in plan.items():
        nm = (LANE - ngs[i] * RV) // 8
        early = max(len(blks) - 2 * nt, 0) if i == 0 else 0
        out[i] = []
        for r, blk in enumerate(blks):
            unit = max(r - early, 0) * (nm + 2) // (len(blks) - early)
            pos = unit if unit <= 2 * QA else max(unit - 2, 2 * QA)
            out[i].append((pos,) + blk)
    return out


def _init_carry(pc_ref, ac_ref):
    pc_ref[...] = jnp.zeros(pc_ref.shape, U32)
    ac_ref[...] = jnp.ones(ac_ref.shape, F32)


def _full_attention(k_ref, qt_ref, vt_ref, ot_ref, kb_ref, z_ref, pc_ref, ac_ref):
    NT = 4
    NSUB = NB // NT
    n = HPI * NSUB * NB

    def keys(i):
        blks = [((i - STAG[t]) // NB + 1) % (HPI * NSUB) for t in range(NT)]
        return [(blk // NSUB, (blk % NSUB) * NT + t) for t, blk in enumerate(blks)]

    assert all(u == 0 for u, _ in keys(n - SKEW)) and keys(n - SKEW) == keys(n - 1)
    assert all(ix % 8 in XREL and ix < n - SKEW for ix in XSTEPS)
    hosted = _plan_vpu(n, NT, keys)
    nslot = [len({_kb_slot(i % NB, x) for i in range(n) for x in range(2 if i in XSTEPS else 1)
                  if any(k[0] == u for k in keys(i))}) for u in range(HPI)]

    def finish(pair, key, acc, lsum, bad):
        o, bad = _normalize(acc, lsum, bad)
        ot_ref[pair, _hrows(key[1], key[0]), :] = _pk(o.astype(BF16))
        return bad

    def tail_step(i, pair, acc):
        vt = _unpk(vt_ref[pair, _hrows(NB - SKEW + i, 0), :])
        if i == 0:
            acc = ac_ref[0:DH, :]
        return acc + jnp.dot(vt, _unpk(pc_ref[i]), preferred_element_type=F32)

    def tail_finish(pair, acc, bad):
        for t, key in enumerate(keys(n - 1)):
            lanes = slice(t * LANE, (t + 1) * LANE)
            bad = finish(pair, key, acc[:, lanes], ac_ref[DH:DH + 8, lanes], bad)
        return bad

    def body(it, bad):
        hp0 = jnp.maximum(it - 1, 0)
        ws, qbs, kbs, accs, lsums, ps, pvs = {}, {}, {}, {}, {}, {}, {}
        remaining = {(u, j): NB for u in range(HPI) for j in range(NB)}
        flags = [bad]

        def setup(js):
            for u, j in js:
                if (u, j) not in ws:
                    q32 = qt_ref[it, _hrows(j, u), :]
                    zq = jnp.zeros_like(q32)
                    ws[(u, j)] = _unpk(_cat(
                        [q32 if rb == u else zq for rb in range(GROUP)], 0))
                    qh = _unpk(q32).astype(F32)
                    qbs[(u, j)] = [jnp.broadcast_to(qh[d:d + 1, :], (8, LANE))
                                   for d in range(DH)]

        def vgroup(i, x):
            if (i, x) not in pvs:
                js = keys(i)
                setup(js)
                slot = _kb_slot(i % NB, x)
                for u in sorted(set(k[0] for k in js)):
                    if (u, slot) not in kbs:
                        kbs[(u, slot)] = [
                            _unpk(kb_ref[u, d, pl.ds(slot * (RV // 2), RV // 2), :]).astype(F32)
                            for d in range(DH)]
                        if sum(k[0] == u for k in kbs) == nslot[u]:
                            _prep_kb(jnp.minimum(it + 1, H // HPI - 1), u, k_ref, kb_ref)
                sv = None
                for d in range(DH):
                    qb = _cat([qbs[key][d] for key in js], 1)
                    t = _cat([kbs[(u, slot)][d] for u, _ in js], 1) * _cat([qb] * (RV // 8), 0)
                    sv = t if sv is None else sv + t
                pvs[(i, x)] = _swap8(jnp.exp2(sv))
            return pvs[(i, x)]

        def qk(i, mid):
            c = i % NB
            js = keys(i)
            setup(js)
            ng = 2 if i in XSTEPS else 1
            nm = (LANE - ng * RV) // 8
            kbl = [k_ref[it, pl.ds(c * (LANE // 2) + bl * 8, 8), :]
                   for bl in range(LANE // 16 - 1, ng - 1, -1)]
            w = _cat([ws[key] for key in js], 1)
            sa = jnp.dot(_unpk(_cat(kbl[:QA], 0)), w, preferred_element_type=F32)
            mid()
            sb = jnp.dot(_unpk(_cat(kbl[QA:], 0)), w, preferred_element_type=F32)
            pm = jnp.exp2(jnp.concatenate([sa, sb], axis=0))
            for t, key in enumerate(js):
                acc = lsums.get(key)
                for b in range(nm + 1):
                    blks = [vgroup(ii, x)[(m // NT) * 8:(m // NT + 1) * 8,
                                          t * LANE:(t + 1) * LANE]
                            for pos, ii, x, m in hosted[i] if pos == b and m % NT == t]
                    if b < nm:
                        blks.append(pm[b * 8:(b + 1) * 8, t * LANE:(t + 1) * LANE])
                    for blk in blks:
                        acc = blk if acc is None else acc + blk
                lsums[key] = acc
            ps[i] = jnp.concatenate(
                [vgroup(i, x) for x in range(ng)]
                + [pm[bl * 8:(bl + 1) * 8] for bl in reversed(range(nm))], axis=0)

        def pv(i):
            js = keys(i)
            p = ps.pop(i)
            for u in sorted(set(k[0] for k in js)):
                ts = [t for t in range(NT) if js[t][0] == u]
                vt = _unpk(vt_ref[it, _hrows(i % NB, u), :]).astype(F32)
                acc = _cat([accs[js[t]] if js[t] in accs else z_ref[:, 0:LANE]
                            for t in ts], 1)
                acc = acc + jnp.dot(vt, p[:, ts[0] * LANE:(ts[-1] + 1) * LANE],
                                    preferred_element_type=F32)
                for m, t in enumerate(ts):
                    key = js[t]
                    accs[key] = acc[:, m * LANE:(m + 1) * LANE]
                    remaining[key] -= 1
                    if remaining[key] == 0:
                        flags[0] = finish(it, key, accs.pop(key), lsums.pop(key), flags[0])

        pacc = [None]

        def tail(i):
            pacc[0] = tail_step(i, hp0, pacc[0])
            if i == SKEW - 1:
                flags[0] = tail_finish(hp0, pacc[0], flags[0])

        for i in range(n):
            qk(i, (lambda: pv(i - SKEW)) if i >= SKEW else (lambda: tail(i)))
        never = pltpu.bitcast(z_ref[0:RV // 2, :], U32) != 0
        for i in range(SKEW):
            pp = _pk(ps.pop(n - SKEW + i).astype(BF16))
            pc_ref[i] = jnp.concatenate(
                [jnp.where(never, pp[RV // 2:RV], pp[:RV // 2]), pp[RV // 2:]], axis=0)
        ac_ref[0:DH, :] = _cat([accs[key] for key in keys(n - 1)], 1)
        ac_ref[DH:DH + 8, :] = _cat([lsums[key] for key in keys(n - 1)], 1)
        return flags[0]

    bad = lax.fori_loop(0, H // HPI, body, jnp.zeros((1, LANE), F32))
    pacc = None
    for i in range(SKEW):
        pacc = tail_step(i, H // HPI - 1, pacc)
    bad = tail_finish(H // HPI - 1, pacc, bad)
    return _cat([bad] * NT, 1)


def _init_bias(bias_ref):
    row = lax.broadcasted_iota(jnp.int32, (LANE, LANE), 0)
    col = lax.broadcasted_iota(jnp.int32, (LANE, LANE), 1)
    bias_ref[0] = jnp.where(row <= col, 0.0, NEG)
    bias_ref[1] = jnp.where(jnp.logical_or(col < row, col >= row + GK), 0.0, NEG)


def _sliding_attention(k_ref, qt_ref, vt_ref, ot_ref, z_ref, pc_ref, ac_ref, bias_ref):
    NH = 4
    W = NH * LANE
    GPB = LANE // GK
    NC = GPB - 1
    MF = -WIN // GK
    M0 = MF + NC
    PL = HPI * DH

    def pv_tile(b, hbase, tiles, acc):
        os = [jnp.dot(_unpk(vt_ref[hbase + u // HPI, _hrows(b, u % HPI), :]),
                      tiles[u], preferred_element_type=F32) for u in range(NH)]
        return (z_ref[...] if acc is None else acc) + jnp.concatenate(os, axis=1)

    def finish(j, hbase, acc, lsum, bad):
        o, bad = _normalize(acc, lsum, bad)
        for u in range(NH):
            ot_ref[hbase + u // HPI, _hrows(j, u % HPI), :] = _pk(
                o[:, u * LANE:(u + 1) * LANE].astype(BF16))
        return bad

    def tail_step(i, hbase, acc):
        tiles = [_unpk(pc_ref[i, :, u * LANE:(u + 1) * LANE]) for u in range(NH)]
        return pv_tile(NB - 3 + i, hbase, tiles, acc)

    def body(it, bad):
        hbase = it * 2
        own = [it * 2 + v for v in range(2)]
        prev = [(p & ~(NP - 1)) + ((p + NP - 1) & (NP - 1)) for p in own]
        lane_q = lax.broadcasted_iota(jnp.int32, (DH // 2, LANE), 1)
        lane_p = lax.broadcasted_iota(jnp.int32, (GK, LANE), 1)
        first_lanes = lax.broadcasted_iota(jnp.int32, (GK // 2, LANE), 1) < PL
        zq = jnp.zeros((DH // 2, LANE), U32)
        flags = [bad]
        lsums, accs, groups = {}, {}, {}

        def krows(p, r0, m):
            return k_ref[p, pl.ds(r0 // 2, m // 2), :]

        def weights(blocks):
            return _unpk(_cat([blocks.get(rb, zq) for rb in range(GROUP)], 0))

        def bias(n, r0):
            return _cat([bias_ref[n, r0:r0 + GK, :]] * NH, 1)

        def probs(j, kcs, ws, biases):
            s = _cat([jnp.dot(_unpk(kcs[v]), _cat(ws[v * HPI:(v + 1) * HPI], 1),
                              preferred_element_type=F32) for v in range(2)], 1)
            s = _swap8(s)
            s = _cat([s[n * GK:(n + 1) * GK] if bs is None
                      else s[n * GK:(n + 1) * GK] + bias(*bs)
                      for n, bs in enumerate(biases)], 0)
            p = jnp.exp2(s)
            part = jnp.sum(p.reshape(p.shape[0] // 8, 8, W), axis=0)
            lsums[j] = part if j not in lsums else lsums[j] + part
            return p

        def passes(j):
            qs = [qt_ref[hbase + u // HPI, _hrows(j, u % HPI), :] for u in range(NH)]
            ws = [weights({u % HPI: qs[u]}) for u in range(NH)]
            k0 = j * LANE

            def shared(m0, m1):
                def run():
                    biases = [(1, NC * GK) if m == M0 else (0, m * GK) if m >= 0 else None
                              for m in range(m0, m1)]
                    kcs = [krows(p, k0 + m0 * GK, (m1 - m0) * GK) for p in own]
                    p = probs(j, kcs, ws, biases)
                    for m in range(m0, m1):
                        groups[(j, m)] = p[(m - m0) * GK:(m - m0 + 1) * GK]
                return run

            def combined(i):
                def run():
                    split = (i + 1) * GK
                    low = lane_q < split
                    wc = [weights({u % HPI: jnp.where(low, qs[u], zq),
                                   u % HPI + HPI: jnp.where(low, zq, qs[u])})
                          for u in range(NH)]
                    kcs = [jnp.where(first_lanes, krows(own[v], k0 + (MF + i) * GK, GK),
                                     krows(prev[v], k0 + split, GK)) for v in range(2)]
                    p = probs(j, kcs, wc, [(1, i * GK)])
                    low = _cat([lane_p < split] * NH, 1)
                    groups[(j, MF + i)] = jnp.where(low, p, 0.0)
                    groups[(j, i + 1)] = jnp.where(low, 0.0, p)
                return run

            if j < 2:
                return [[shared(m, m + GPB // 2)] for m in range(-GPB * j, GPB, GPB // 2)]
            cuts = [M0 + (n * (1 - M0)) // 3 for n in range(4)]
            ccut = [(n * NC) // 3 for n in range(4)]
            return [[combined(i) for i in range(ccut[n], ccut[n + 1])]
                    + [shared(cuts[n], cuts[n + 1])] for n in range(3)]

        def tile(j, b):
            p = _cat([groups.pop((j, m))
                      for m in range(GPB * (b - j), GPB * (b - j + 1))], 0)
            return [p[:, u * LANE:(u + 1) * LANE].astype(BF16) for u in range(NH)]

        def pv(j, b):
            accs[j] = pv_tile(b, hbase, tile(j, b), accs.get(j))
            if b == j:
                flags[0] = finish(j, hbase, accs.pop(j), lsums.pop(j), flags[0])

        hprev = jnp.maximum(hbase - 2, 0)

        def tail(i):
            accs[-1] = tail_step(i, hprev, accs.get(-1))
            if i == 2:
                flags[0] = finish(NB - 1, hprev, accs.pop(-1), ac_ref[DH:DH + 8, :], flags[0])

        pending = [(0, lambda i=i: tail(i)) for i in range(3)]
        slot = 0
        for j in range(NB):
            for runs in passes(j):
                for run in runs:
                    run()
                if pending and pending[0][0] <= slot:
                    pending.pop(0)[1]()
                slot += 1
            if j < NB - 1:
                pending += [(slot + LAG_A, lambda j=j, b=b: pv(j, b))
                            for b in range(max(j - 2, 0), j + 1)]
        for _, job in pending:
            job()
        for i in range(3):
            for u, t in enumerate(tile(NB - 1, NB - 3 + i)):
                pc_ref[i, :, u * LANE:(u + 1) * LANE] = _pk(t)
        ac_ref[DH:DH + 8, :] = lsums.pop(NB - 1)
        return flags[0]

    bad = lax.fori_loop(0, H // NH, body, jnp.zeros((1, W), F32))
    pacc = None
    for i in range(3):
        pacc = tail_step(i, H // HPI - 2, pacc)
    return finish(NB - 1, H // HPI - 2, pacc, ac_ref[DH:DH + 8, :], bad)


def _safe_attention(k_ref, qt_ref, vt_ref, ot_ref, sliding):
    NKB = (WIN // LANE + 1) if sliding else NB
    NK = NKB * LANE

    def body(it, carry):
        h = it >> 4
        j = it & (NB - 1)
        pair, u = h >> 1, h & 1
        cb = jnp.maximum(j - WIN // LANE, 0) if sliding else 0
        k0h = _mo(cb * (LANE // 2), LANE // 2)
        q32 = qt_ref[pair, _hrows(j, u), :]
        w = _head_weights(_cat([q32] * GROUP, 0), u)
        kc = _unpk(k_ref[pair, pl.ds(k0h, NK // 2), :])
        s = _swap8(jnp.dot(kc, w, preferred_element_type=F32))
        if sliding:
            kpos = cb * LANE + lax.broadcasted_iota(jnp.int32, s.shape, 0)
            qpos = j * LANE + lax.broadcasted_iota(jnp.int32, s.shape, 1)
            d = qpos - kpos
            s = jnp.where(jnp.logical_and(d >= 0, d < WIN), s, -1e9)
        m = jnp.max(s, axis=0, keepdims=True)
        p = jnp.exp2(s - m)
        l = jnp.sum(p, axis=0, keepdims=True)
        p = (p * (1.0 / l)).astype(BF16)
        vt = _unpk(_cat([vt_ref[pair, _hrows(cb + i, u), :] for i in range(NKB)], 1))
        o = jnp.dot(vt, p, preferred_element_type=F32)
        ot_ref[pair, _hrows(j, u), :] = _pk(o.astype(BF16))
        return carry

    lax.fori_loop(0, H * NB, body, 0)


def _attention(k_ref, qt_ref, vt_ref, ot_ref, kb_ref, z_ref, pc_ref, ac_ref, bias_ref,
               vflag_ref, sliding):
    if sliding:
        bad = _sliding_attention(k_ref, qt_ref, vt_ref, ot_ref, z_ref, pc_ref, ac_ref, bias_ref)
    else:
        bad = _full_attention(k_ref, qt_ref, vt_ref, ot_ref, kb_ref, z_ref, pc_ref, ac_ref)

    bad = jnp.maximum(bad, jnp.max(vflag_ref[...].reshape(S // TM * 8, TM), axis=0, keepdims=True))

    @pl.when(jnp.max(bad) > 0.0)
    def _():
        _safe_attention(k_ref, qt_ref, vt_ref, ot_ref, sliding)


def _layernorm(x):
    m = jnp.mean(x, axis=-1, keepdims=True)
    xc = x - m
    v = jnp.mean(xc * xc, axis=-1, keepdims=True)
    return (xc * lax.rsqrt(v + LN_EPS)).astype(BF16)


def _project_k(xn, i, wk, k_ref, g0=0, copies=NP):
    k = _swap8(jnp.dot(xn, wk, preferred_element_type=F32))
    for g in range(wk.shape[1] // LANE):
        kg = _pk(k[:, g * LANE:(g + 1) * LANE].astype(BF16))
        for p in range(copies):
            k_ref[(g0 + g) * NP + p, pl.ds(_mo(i * (TM // 2), TM // 2), TM // 2), :] = (
                pltpu.roll(kg, LANE - p * HPI * DH, 1) if p else kg)


def _project_qv(xn, i, wt, qt_ref, vt_ref, vflag_ref):
    qv = lax.dot_general(wt, xn, (((1,), (1,)), ((), ())),
                         preferred_element_type=F32)
    for t in range(TM // LANE):
        j = i * (TM // LANE) + t
        qt = _pk((qv[:D, t * LANE:(t + 1) * LANE] * QSCALE).astype(BF16))
        vt = _pk(qv[D:, t * LANE:(t + 1) * LANE].astype(BF16))
        r = pl.ds(_mo(j * PR, PR), PR)
        for p in range(H // HPI):
            qt_ref[p, r, :] = qt[p * PR:(p + 1) * PR]
            vt_ref[p, r, :] = vt[p * PR:(p + 1) * PR]
    big = jnp.where(jnp.abs(qv[D:]) < V_HI, 0.0, 1.0)
    vflag_ref[i] = jnp.max(big.reshape(D // 8, 8, TM), axis=0)


def _project_out(i, ot_ref, wo, tm=TM):
    ot = _unpk(_cat([_cat([ot_ref[p, pl.ds(_mo((i * (tm // LANE) + t) * PR, PR), PR), :]
                           for p in range(H // HPI)], 0)
                     for t in range(tm // LANE)], 1))
    return lax.dot_general(ot, wo, (((0,), (0,)), ((), ())),
                           preferred_element_type=F32)


def _kernel(x_hbm, wa_hbm, woa_hbm, wb_hbm, wob_hbm, o_hbm,
            xb_ref, w_ref, wo_ref, wt_ref, xres_ref, xn_ref,
            k_ref, qt_ref, vt_ref, ot_ref, kb_ref, z_ref, pc_ref, ac_ref, bias_ref, vflag_ref, sems):
    nchunk = S // TM

    def rows(i):
        return pl.ds(_mo(i * TM, TM), TM)

    x_cp = [pltpu.make_async_copy(x_hbm.at[rows(i)], xb_ref.at[rows(i)], sems.at[i])
            for i in range(nchunk)]
    wa_cp = [pltpu.make_async_copy(wa_hbm.at[:, pl.ds(n * D, D)], w_ref.at[0, n],
                                   sems.at[nchunk + n]) for n in range(3)]
    wb_cp = [pltpu.make_async_copy(wb_hbm.at[:, pl.ds(n * D, D)], w_ref.at[1, n],
                                   sems.at[nchunk + 3 + n]) for n in range(3)]
    wo_cp = [pltpu.make_async_copy(src, wo_ref.at[n], sems.at[nchunk + 6 + n])
             for n, src in enumerate((woa_hbm, wob_hbm))]
    for cp in (x_cp[0], wa_cp[1], *x_cp[1:], wa_cp[0], wa_cp[2],
               wb_cp[0], wb_cp[2], wb_cp[1], *wo_cp):
        cp.start()

    z_ref[...] = jnp.zeros(z_ref.shape, F32)
    _init_bias(bias_ref)
    _init_carry(pc_ref, ac_ref)

    def normalize(i, x):
        xres_ref[rows(i), :] = x
        return _layernorm(x)

    def project_qv(i, xn, kind):
        _project_qv(xn, i, _unpk(wt_ref[kind]), qt_ref, vt_ref, vflag_ref)

    def stash(i):
        xn = normalize(i, xb_ref[rows(i), :].astype(F32))
        xn_ref[i] = _pk(xn)
        return xn

    def first_k(xn, i, half):
        _project_k(xn, i, w_ref[0, 1, :, half * (D // 2):(half + 1) * (D // 2)], k_ref,
                   half * (NG // 2), 1)

    x_cp[0].wait()
    xn0 = stash(0)
    wa_cp[1].wait()
    first_k(xn0, 0, 0)
    x_cp[1].wait()
    first_k(xn0, 0, 1)
    xn1 = stash(1)
    first_k(xn1, 1, 0)
    x_cp[2].wait()
    x_cp[3].wait()
    first_k(xn1, 1, 1)
    xn2 = stash(2)
    _project_k(xn2, 2, w_ref[0, 1], k_ref, 0, 1)
    xn3 = stash(3)
    first_k(xn3, 3, 0)
    wa_cp[0].wait()
    wa_cp[2].wait()
    first_k(xn3, 3, 1)
    wt_ref[0, 0:D // 2, :] = _pk(w_ref[0, 0].T)
    wt_ref[0, D // 2:D, :] = _pk(w_ref[0, 2].T)

    def first_qv(it, c):
        n = 2 * it
        pltpu.make_async_copy(wb_hbm.at[:, pl.ds(pl.multiple_of(n * D, D), D)],
                              w_ref.at[1, n], sems.at[nchunk + 3 + n]).wait()
        for i in (2 * it, 2 * it + 1):
            project_qv(i, _unpk(xn_ref[i]), 0)
        r = pl.ds(pl.multiple_of(it * TM, TM), TM)
        for g in range(NG):
            kg = k_ref[g * NP, r, :]
            for p in range(1, NP):
                k_ref[g * NP + p, r, :] = pltpu.roll(kg, LANE - p * HPI * DH, 1)
        wt_ref[1, pl.ds(pl.multiple_of(it * (D // 2), D // 2), D // 2), :] = _pk(w_ref[1, n].T)
        return c

    lax.fori_loop(0, 2, first_qv, 0)
    for cp in (wb_cp[1], *wo_cp):
        cp.wait()

    def layer(t, carry):
        cur = t & 1

        @pl.when(cur == 0)
        def _():
            _attention(k_ref, qt_ref, vt_ref, ot_ref, kb_ref, z_ref, pc_ref, ac_ref, bias_ref,
                       vflag_ref, sliding=True)

        @pl.when(cur == 1)
        def _():
            _attention(k_ref, qt_ref, vt_ref, ot_ref, kb_ref, z_ref, pc_ref, ac_ref, bias_ref,
                       vflag_ref, sliding=False)

        @pl.when(t < 3)
        def _():
            nxt = 1 - cur

            def resid(i):
                xns = []
                for m in range(TM // TR):
                    r = pl.ds(pl.multiple_of(i * TM + m * TR, TR), TR)
                    x = xres_ref[r, :] + _project_out(i * (TM // TR) + m, ot_ref, wo_ref[cur], TR)
                    xres_ref[r, :] = x
                    xns.append(_layernorm(x))
                return _cat(xns, 0)

            def half(it, c):
                a, b = 2 * it, 2 * it + 1
                xa = resid(a)
                xb = resid(b)
                _project_k(xa, a, w_ref[nxt, 1], k_ref)
                _project_k(xb, b, w_ref[nxt, 1], k_ref)
                project_qv(a, xa, nxt)
                project_qv(b, xb, nxt)
                for u in range(HPI):
                    _prep_kb(0, u, k_ref, kb_ref, it)
                _init_carry(pc_ref, ac_ref)
                return c

            lax.fori_loop(0, nchunk // 2, half, 0)
        return carry

    lax.fori_loop(0, 4, layer, 0)

    o_cp = [pltpu.make_async_copy(xb_ref.at[pl.ds(i * TR, TR)], o_hbm.at[pl.ds(i * TR, TR)],
                                  sems.at[i]) for i in range(S // TR)]
    for i in range(S // TR):
        x = xres_ref[pl.ds(i * TR, TR), :] + _project_out(i, ot_ref, wo_ref[1], TR)
        xb_ref[pl.ds(i * TR, TR), :] = x.astype(BF16)
        o_cp[i].start()
    for cp in o_cp:
        cp.wait()


@jax.jit
def pallas_interleave_layers__sliding_block__mha_block__prompt_kernel(
    A_x: jax.Array,
    A_wqkv: jax.Array,
    A_wo: jax.Array,
    B_x: jax.Array,
    B_wqkv: jax.Array,
    B_wo: jax.Array,
):
    del B_x
    x = A_x.reshape(S, D)
    any_spec = pl.BlockSpec(memory_space=pl.ANY)
    out = pl.pallas_call(
        _kernel,
        out_shape=jax.ShapeDtypeStruct((S, D), A_x.dtype),
        in_specs=[any_spec] * 5,
        out_specs=any_spec,
        scratch_shapes=[
            pltpu.VMEM((S, D), BF16),
            pltpu.VMEM((2, 3, D, D), BF16),
            pltpu.VMEM((2, D, D), BF16),
            pltpu.VMEM((2, D, D), U32),
            pltpu.VMEM((S, D), F32),
            pltpu.VMEM((S // TM, TM // 2, D), U32),
            pltpu.VMEM((NG * NP, S // 2, LANE), U32),
            pltpu.VMEM((H // HPI, NB * PR, LANE), U32),
            pltpu.VMEM((H // HPI, NB * PR, LANE), U32),
            pltpu.VMEM((H // HPI, NB * PR, LANE), U32),
            pltpu.VMEM((HPI, DH, 2 * KB_HALF * RV // 2, LANE), U32),
            pltpu.VMEM((DH, 4 * LANE), F32),
            pltpu.VMEM((3, LANE // 2, 4 * LANE), U32),
            pltpu.VMEM((DH + 8, 4 * LANE), F32),
            pltpu.VMEM((2, LANE, LANE), F32),
            pltpu.VMEM((S // TM, 8, TM), F32),
            pltpu.SemaphoreType.DMA((max(S // TM + 8, S // TR),)),
        ],
        compiler_params=pltpu.CompilerParams(vmem_limit_bytes=100 * 1024 * 1024),
    )(x, A_wqkv, A_wo, B_wqkv, B_wo)
    return out.reshape(A_x.shape)
```

```python
import math

import jax
import jax.numpy as jnp
from jax import lax
import jax.experimental.pallas as pl
import jax.experimental.pallas.tpu as pltpu

S = 2048
D = 512
H = 32
DH = D // H
WIN = 256
LANE = 128
GROUP = LANE // DH
NG = D // LANE
NB = S // LANE
QSCALE = (DH ** -0.5) * math.log2(math.e)
LN_EPS = 1e-5
L_LO = 2.0 ** -60
L_HI = 2.0 ** 60
V_HI = 2.0 ** 60
NEG = -1e30

TM = 512
TR = 128
GK = 16
LAG_A = 2
HPI = 2
PR = HPI * DH // 2
NP = GROUP // HPI
RV = 16
QA = 2
SKEW = 2
STAG = (11, 12, 13, 14)
XREL = (2, 5, 7)
XSTEPS = (18, 21, 23, 26, 34, 37, 39, 42, 50, 53, 55, 58, 74, 82, 85, 87, 90, 98, 101, 103, 106, 114)
KB_HALF = 12
BORDER = (0, 4, 1, 5, 2, 6, 3, 7)
UTIL_MIN = 188
COST_Q = 60
COST_K = 56
COST_F = 10
COST_X = 30
XLU_STEPS = 14
START_SLOTS = 400
F32 = jnp.float32
BF16 = jnp.bfloat16
U32 = jnp.uint32


def _cat(xs, axis):
    return xs[0] if len(xs) == 1 else jnp.concatenate(xs, axis=axis)


def _pk(x):
    return pltpu.bitcast(x, U32)


def _unpk(x):
    return pltpu.bitcast(x, BF16)


def _swap8(x):
    y = x.reshape(x.shape[0] // 16, 2, 8, x.shape[1])
    return jnp.concatenate([y[:, 1:2], y[:, 0:1]], axis=1).reshape(x.shape)


def _hrows(j, u):
    return pl.ds(_mo((j * HPI + u) * (DH // 2), DH // 2), DH // 2)


def _head_weights(q32, r):
    rows = lax.broadcasted_iota(jnp.int32, q32.shape, 0) >> 3
    return pltpu.bitcast(jnp.where(rows == r, q32, jnp.uint32(0)), BF16)


def _normalize(acc, lsum, bad):
    l = jnp.sum(lsum, axis=0, keepdims=True)
    r = pl.reciprocal(l, approx=True)
    r = r * (2.0 - l * r)
    ok = jnp.logical_and(l >= L_LO, l <= L_HI)
    return acc * r, jnp.where(ok, bad, 1.0)


def _mo(x, m):
    return x if isinstance(x, int) else pl.multiple_of(x, m)


def _kb_slot(c, x):
    return (c // 8) * KB_HALF + (NB // 2 + XREL.index(c % 8) if x else c % 8)


def _prep_kb(pair, u, k_ref, kb_ref, half=None):
    if half is None:
        grps = [(c, 0) for c in range(NB)] + sorted({(i % NB, 1) for i in XSTEPS})
        half = 0
    else:
        grps = [(c, 0) for c in range(NB // 2)] + [(c, 1) for c in XREL]
    kk = _cat([k_ref[pair, pl.ds(_mo(half * (S // 4) + c * (LANE // 2) + x * (RV // 2), 8),
                                 RV // 2), :] for c, x in grps], 0)
    runs = []
    for n, (c, x) in enumerate(grps):
        if runs and runs[-1][1] + runs[-1][2] == _kb_slot(c, x):
            runs[-1][2] += 1
        else:
            runs.append([n, _kb_slot(c, x), 1])
    for d in range(DH):
        b = jnp.broadcast_to(kk[:, u * DH + d:u * DH + d + 1], kk.shape)
        for n, slot, cnt in runs:
            r0 = _mo((half * KB_HALF + slot) * (RV // 2), 8)
            kb_ref[u, d, pl.ds(r0, cnt * (RV // 2)), :] = (
                b[n * (RV // 2):(n + cnt) * (RV // 2)])


def _plan_vpu(n, nt, keys):
    cost = 2 * DH + 1
    ngs = [2 if i in XSTEPS else 1 for i in range(n)]
    other, seen = [], set()
    for i in range(n):
        load = 2 * nt * (LANE - ngs[i] * RV) // 8 + 10
        new = {("q",) + k for k in keys(i)}
        load += COST_Q * len(new - seen)
        kbn = {("k", u, _kb_slot(i % NB, x)) for u, _ in keys(i) for x in range(ngs[i])}
        load += COST_K * len(kbn - seen)
        seen |= new | kbn
        if i > SKEW:
            load += COST_F * sum(a != b for a, b in zip(keys(i - SKEW - 1), keys(i - SKEW)))
        if i >= n - XLU_STEPS:
            load += COST_X
        other.append(load)

    def attempt(util):
        pool, frac, plan, ok = [], 0.0, {}, True
        for i in reversed(range(n)):
            pool += [(i, x, m) for x in range(ngs[i]) for m in BORDER]
            cap = util * 4 * (LANE + 16 - ngs[i] * RV) - other[i] + frac
            if i == 0:
                cap += START_SLOTS
            k = max(int(cap // cost), 0)
            frac = cap - k * cost
            must = [blk for blk in pool
                    if i == 0 or keys(i - 1)[blk[2] % nt] != keys(blk[0])[blk[2] % nt]]
            ok = ok and len(must) <= k + 1
            rest = [blk for blk in pool if blk not in must]
            rest.sort(key=lambda blk: blk[:2] != (i, 0))
            take = must + rest[:max(k - len(must), 0)]
            pool = [blk for blk in pool if blk not in take]
            plan[i] = sorted(take, key=lambda blk: (blk[0], blk[1], BORDER.index(blk[2])))
        return ok, plan

    util = next(v / 200 for v in range(UTIL_MIN, 240) if attempt(v / 200)[0])
    plan = attempt(util)[1]
    out = {}
    for i, blks in plan.items():
        nm = (LANE - ngs[i] * RV) // 8
        early = max(len(blks) - 2 * nt, 0) if i == 0 else 0
        out[i] = []
        for r, blk in enumerate(blks):
            unit = max(r - early, 0) * (nm + 2) // (len(blks) - early)
            pos = unit if unit <= 2 * QA else max(unit - 2, 2 * QA)
            out[i].append((pos,) + blk)
    return out


def _init_carry(pc_ref, ac_ref):
    pc_ref[...] = jnp.zeros(pc_ref.shape, U32)
    ac_ref[...] = jnp.ones(ac_ref.shape, F32)


def _full_attention(k_ref, qt_ref, vt_ref, ot_ref, kb_ref, z_ref, pc_ref, ac_ref):
    NT = 4
    NSUB = NB // NT
    n = HPI * NSUB * NB

    def keys(i):
        blks = [((i - STAG[t]) // NB + 1) % (HPI * NSUB) for t in range(NT)]
        return [(blk // NSUB, (blk % NSUB) * NT + t) for t, blk in enumerate(blks)]

    assert all(u == 0 for u, _ in keys(n - SKEW)) and keys(n - SKEW) == keys(n - 1)
    assert all(ix % 8 in XREL and ix < n - SKEW for ix in XSTEPS)
    hosted = _plan_vpu(n, NT, keys)
    nslot = [len({_kb_slot(i % NB, x) for i in range(n) for x in range(2 if i in XSTEPS else 1)
                  if any(k[0] == u for k in keys(i))}) for u in range(HPI)]

    def finish(pair, key, acc, lsum, bad):
        o, bad = _normalize(acc, lsum, bad)
        ot_ref[pair, _hrows(key[1], key[0]), :] = _pk(o.astype(BF16))
        return bad

    def tail_step(i, pair, acc):
        vt = _unpk(vt_ref[pair, _hrows(NB - SKEW + i, 0), :])
        if i == 0:
            acc = ac_ref[0:DH, :]
        return acc + jnp.dot(vt, _unpk(pc_ref[i]), preferred_element_type=F32)

    def tail_finish(pair, acc, bad):
        for t, key in enumerate(keys(n - 1)):
            lanes = slice(t * LANE, (t + 1) * LANE)
            bad = finish(pair, key, acc[:, lanes], ac_ref[DH:DH + 8, lanes], bad)
        return bad

    def body(it, bad):
        hp0 = jnp.maximum(it - 1, 0)
        ws, qbs, kbs, accs, lsums, ps, pvs, wide = {}, {}, {}, {}, {}, {}, {}, {}
        remaining = {(u, j): NB for u in range(HPI) for j in range(NB)}
        lw = [None]
        flags = [bad]

        def setup(js):
            for u, j in js:
                if (u, j) not in ws:
                    q32 = qt_ref[it, _hrows(j, u), :]
                    zq = jnp.zeros_like(q32)
                    ws[(u, j)] = _unpk(_cat(
                        [q32 if rb == u else zq for rb in range(GROUP)], 0))
                    qh = _unpk(q32).astype(F32)
                    qbs[(u, j)] = [jnp.broadcast_to(qh[d:d + 1, :], (8, LANE))
                                   for d in range(DH)]

        def vgroup(i, x):
            if (i, x) not in pvs:
                js = keys(i)
                setup(js)
                slot = _kb_slot(i % NB, x)
                for u in sorted(set(k[0] for k in js)):
                    if (u, slot) not in kbs:
                        kbs[(u, slot)] = [
                            _unpk(kb_ref[u, d, pl.ds(slot * (RV // 2), RV // 2), :]).astype(F32)
                            for d in range(DH)]
                        if sum(k[0] == u for k in kbs) == nslot[u]:
                            _prep_kb(jnp.minimum(it + 1, H // HPI - 1), u, k_ref, kb_ref)
                qkey, kkey = tuple(js), (slot,) + tuple(u for u, _ in js)
                if qkey not in wide:
                    wide[qkey] = [_cat([_cat([qbs[key][d] for key in js], 1)] * (RV // 8), 0)
                                  for d in range(DH)]
                if kkey not in wide:
                    wide[kkey] = [_cat([kbs[(u, slot)][d] for u, _ in js], 1)
                                  for d in range(DH)]
                sv = None
                for d in range(DH):
                    t = wide[kkey][d] * wide[qkey][d]
                    sv = t if sv is None else sv + t
                pvs[(i, x)] = _swap8(jnp.exp2(sv))
            return pvs[(i, x)]

        def qk(i, mid):
            c = i % NB
            js = keys(i)
            setup(js)
            ng = 2 if i in XSTEPS else 1
            nm = (LANE - ng * RV) // 8
            kbl = [k_ref[it, pl.ds(c * (LANE // 2) + bl * 8, 8), :]
                   for bl in range(LANE // 16 - 1, ng - 1, -1)]
            w = _cat([ws[key] for key in js], 1)
            sa = jnp.dot(_unpk(_cat(kbl[:QA], 0)), w, preferred_element_type=F32)
            mid()
            sb = jnp.dot(_unpk(_cat(kbl[QA:], 0)), w, preferred_element_type=F32)
            pm = jnp.exp2(jnp.concatenate([sa, sb], axis=0))
            rows = [pm[b * 8:(b + 1) * 8] for b in range(nm)]
            fresh = [key not in lsums for key in js]
            if i == 0 or keys(i - 1) != js:
                lw[0] = _cat([rows[0][:, t * LANE:(t + 1) * LANE] if fresh[t] else lsums[key]
                              for t, key in enumerate(js)], 1)

            def add_tile(t, blk):
                parts = [lw[0][:, t * LANE:(t + 1) * LANE] + blk]
                if t > 0:
                    parts.insert(0, lw[0][:, :t * LANE])
                if t < NT - 1:
                    parts.append(lw[0][:, (t + 1) * LANE:])
                lw[0] = jnp.concatenate(parts, axis=1)

            for b in range(nm + 1):
                for pos, ii, x, m in hosted[i]:
                    if pos == b:
                        t = m % NT
                        add_tile(t, vgroup(ii, x)[(m // NT) * 8:(m // NT + 1) * 8,
                                                  t * LANE:(t + 1) * LANE])
                if b == 0 and any(fresh):
                    for t in range(NT):
                        if not fresh[t]:
                            add_tile(t, rows[0][:, t * LANE:(t + 1) * LANE])
                elif b < nm:
                    lw[0] = lw[0] + rows[b]
            if i == n - 1 or keys(i + 1) != js or any(fresh):
                lsums.update((key, lw[0][:, t * LANE:(t + 1) * LANE])
                             for t, key in enumerate(js))
            ps[i] = jnp.concatenate(
                [vgroup(i, x) for x in range(ng)] + rows[::-1], axis=0)

        def pv(i):
            js = keys(i)
            p = ps.pop(i)
            for u in sorted(set(k[0] for k in js)):
                ts = [t for t in range(NT) if js[t][0] == u]
                vt = _unpk(vt_ref[it, _hrows(i % NB, u), :]).astype(F32)
                acc = _cat([accs[js[t]] if js[t] in accs else z_ref[:, 0:LANE]
                            for t in ts], 1)
                acc = acc + jnp.dot(vt, p[:, ts[0] * LANE:(ts[-1] + 1) * LANE],
                                    preferred_element_type=F32)
                for m, t in enumerate(ts):
                    key = js[t]
                    accs[key] = acc[:, m * LANE:(m + 1) * LANE]
                    remaining[key] -= 1
                    if remaining[key] == 0:
                        flags[0] = finish(it, key, accs.pop(key), lsums.pop(key), flags[0])

        pacc = [None]

        def tail(i):
            pacc[0] = tail_step(i, hp0, pacc[0])
            if i == SKEW - 1:
                flags[0] = tail_finish(hp0, pacc[0], flags[0])

        for i in range(n):
            qk(i, (lambda: pv(i - SKEW)) if i >= SKEW else (lambda: tail(i)))
        never = pltpu.bitcast(z_ref[0:RV // 2, :], U32) != 0
        for i in range(SKEW):
            pp = _pk(ps.pop(n - SKEW + i).astype(BF16))
            pc_ref[i] = jnp.concatenate(
                [jnp.where(never, pp[RV // 2:RV], pp[:RV // 2]), pp[RV // 2:]], axis=0)
        ac_ref[0:DH, :] = _cat([accs[key] for key in keys(n - 1)], 1)
        ac_ref[DH:DH + 8, :] = _cat([lsums[key] for key in keys(n - 1)], 1)
        return flags[0]

    bad = lax.fori_loop(0, H // HPI, body, jnp.zeros((1, LANE), F32))
    pacc = None
    for i in range(SKEW):
        pacc = tail_step(i, H // HPI - 1, pacc)
    bad = tail_finish(H // HPI - 1, pacc, bad)
    return _cat([bad] * NT, 1)


def _init_bias(bias_ref):
    row = lax.broadcasted_iota(jnp.int32, (LANE, LANE), 0)
    col = lax.broadcasted_iota(jnp.int32, (LANE, LANE), 1)
    bias_ref[0] = jnp.where(row <= col, 0.0, NEG)
    bias_ref[1] = jnp.where(jnp.logical_or(col < row, col >= row + GK), 0.0, NEG)


def _sliding_attention(k_ref, qt_ref, vt_ref, ot_ref, z_ref, pc_ref, ac_ref, bias_ref):
    NH = 4
    W = NH * LANE
    GPB = LANE // GK
    NC = GPB - 1
    MF = -WIN // GK
    M0 = MF + NC
    PL = HPI * DH

    def pv_tile(b, hbase, tiles, acc):
        os = [jnp.dot(_unpk(vt_ref[hbase + u // HPI, _hrows(b, u % HPI), :]),
                      tiles[u], preferred_element_type=F32) for u in range(NH)]
        return (z_ref[...] if acc is None else acc) + jnp.concatenate(os, axis=1)

    def finish(j, hbase, acc, lsum, bad):
        o, bad = _normalize(acc, lsum, bad)
        for u in range(NH):
            ot_ref[hbase + u // HPI, _hrows(j, u % HPI), :] = _pk(
                o[:, u * LANE:(u + 1) * LANE].astype(BF16))
        return bad

    def tail_step(i, hbase, acc):
        tiles = [_unpk(pc_ref[i, :, u * LANE:(u + 1) * LANE]) for u in range(NH)]
        return pv_tile(NB - 3 + i, hbase, tiles, acc)

    def body(it, bad):
        hbase = it * 2
        own = [it * 2 + v for v in range(2)]
        prev = [(p & ~(NP - 1)) + ((p + NP - 1) & (NP - 1)) for p in own]
        lane_q = lax.broadcasted_iota(jnp.int32, (DH // 2, LANE), 1)
        lane_p = lax.broadcasted_iota(jnp.int32, (GK, LANE), 1)
        first_lanes = lax.broadcasted_iota(jnp.int32, (GK // 2, LANE), 1) < PL
        zq = jnp.zeros((DH // 2, LANE), U32)
        flags = [bad]
        lsums, accs, groups = {}, {}, {}

        def krows(p, r0, m):
            return k_ref[p, pl.ds(r0 // 2, m // 2), :]

        def weights(blocks):
            return _unpk(_cat([blocks.get(rb, zq) for rb in range(GROUP)], 0))

        def bias(n, r0):
            return _cat([bias_ref[n, r0:r0 + GK, :]] * NH, 1)

        def probs(j, kcs, ws, biases):
            s = _cat([jnp.dot(_unpk(kcs[v]), _cat(ws[v * HPI:(v + 1) * HPI], 1),
                              preferred_element_type=F32) for v in range(2)], 1)
            s = _swap8(s)
            s = _cat([s[n * GK:(n + 1) * GK] if bs is None
                      else s[n * GK:(n + 1) * GK] + bias(*bs)
                      for n, bs in enumerate(biases)], 0)
            p = jnp.exp2(s)
            part = jnp.sum(p.reshape(p.shape[0] // 8, 8, W), axis=0)
            lsums[j] = part if j not in lsums else lsums[j] + part
            return p

        def passes(j):
            qs = [qt_ref[hbase + u // HPI, _hrows(j, u % HPI), :] for u in range(NH)]
            ws = [weights({u % HPI: qs[u]}) for u in range(NH)]
            k0 = j * LANE

            def shared(m0, m1):
                def run():
                    biases = [(1, NC * GK) if m == M0 else (0, m * GK) if m >= 0 else None
                              for m in range(m0, m1)]
                    kcs = [krows(p, k0 + m0 * GK, (m1 - m0) * GK) for p in own]
                    p = probs(j, kcs, ws, biases)
                    for m in range(m0, m1):
                        groups[(j, m)] = p[(m - m0) * GK:(m - m0 + 1) * GK]
                return run

            def combined(i):
                def run():
                    split = (i + 1) * GK
                    low = lane_q < split
                    wc = [weights({u % HPI: jnp.where(low, qs[u], zq),
                                   u % HPI + HPI: jnp.where(low, zq, qs[u])})
                          for u in range(NH)]
                    kcs = [jnp.where(first_lanes, krows(own[v], k0 + (MF + i) * GK, GK),
                                     krows(prev[v], k0 + split, GK)) for v in range(2)]
                    p = probs(j, kcs, wc, [(1, i * GK)])
                    low = _cat([lane_p < split] * NH, 1)
                    groups[(j, MF + i)] = jnp.where(low, p, 0.0)
                    groups[(j, i + 1)] = jnp.where(low, 0.0, p)
                return run

            if j < 2:
                return [[shared(m, m + GPB // 2)] for m in range(-GPB * j, GPB, GPB // 2)]
            cuts = [M0 + (n * (1 - M0)) // 3 for n in range(4)]
            ccut = [(n * NC) // 3 for n in range(4)]
            return [[combined(i) for i in range(ccut[n], ccut[n + 1])]
                    + [shared(cuts[n], cuts[n + 1])] for n in range(3)]

        def tile(j, b):
            p = _cat([groups.pop((j, m))
                      for m in range(GPB * (b - j), GPB * (b - j + 1))], 0)
            return [p[:, u * LANE:(u + 1) * LANE].astype(BF16) for u in range(NH)]

        def pv(j, b):
            accs[j] = pv_tile(b, hbase, tile(j, b), accs.get(j))
            if b == j:
                flags[0] = finish(j, hbase, accs.pop(j), lsums.pop(j), flags[0])

        hprev = jnp.maximum(hbase - 2, 0)

        def tail(i):
            accs[-1] = tail_step(i, hprev, accs.get(-1))
            if i == 2:
                flags[0] = finish(NB - 1, hprev, accs.pop(-1), ac_ref[DH:DH + 8, :], flags[0])

        pending = [(0, lambda i=i: tail(i)) for i in range(3)]
        slot = 0
        for j in range(NB):
            for runs in passes(j):
                for run in runs:
                    run()
                if pending and pending[0][0] <= slot:
                    pending.pop(0)[1]()
                slot += 1
            if j < NB - 1:
                pending += [(slot + LAG_A, lambda j=j, b=b: pv(j, b))
                            for b in range(max(j - 2, 0), j + 1)]
        for _, job in pending:
            job()
        for i in range(3):
            for u, t in enumerate(tile(NB - 1, NB - 3 + i)):
                pc_ref[i, :, u * LANE:(u + 1) * LANE] = _pk(t)
        ac_ref[DH:DH + 8, :] = lsums.pop(NB - 1)
        return flags[0]

    bad = lax.fori_loop(0, H // NH, body, jnp.zeros((1, W), F32))
    pacc = None
    for i in range(3):
        pacc = tail_step(i, H // HPI - 2, pacc)
    return finish(NB - 1, H // HPI - 2, pacc, ac_ref[DH:DH + 8, :], bad)


def _safe_attention(k_ref, qt_ref, vt_ref, ot_ref, sliding):
    NKB = (WIN // LANE + 1) if sliding else NB
    NK = NKB * LANE

    def body(it, carry):
        h = it >> 4
        j = it & (NB - 1)
        pair, u = h >> 1, h & 1
        cb = jnp.maximum(j - WIN // LANE, 0) if sliding else 0
        k0h = _mo(cb * (LANE // 2), LANE // 2)
        q32 = qt_ref[pair, _hrows(j, u), :]
        w = _head_weights(_cat([q32] * GROUP, 0), u)
        kc = _unpk(k_ref[pair, pl.ds(k0h, NK // 2), :])
        s = _swap8(jnp.dot(kc, w, preferred_element_type=F32))
        if sliding:
            kpos = cb * LANE + lax.broadcasted_iota(jnp.int32, s.shape, 0)
            qpos = j * LANE + lax.broadcasted_iota(jnp.int32, s.shape, 1)
            d = qpos - kpos
            s = jnp.where(jnp.logical_and(d >= 0, d < WIN), s, -1e9)
        m = jnp.max(s, axis=0, keepdims=True)
        p = jnp.exp2(s - m)
        l = jnp.sum(p, axis=0, keepdims=True)
        p = (p * (1.0 / l)).astype(BF16)
        vt = _unpk(_cat([vt_ref[pair, _hrows(cb + i, u), :] for i in range(NKB)], 1))
        o = jnp.dot(vt, p, preferred_element_type=F32)
        ot_ref[pair, _hrows(j, u), :] = _pk(o.astype(BF16))
        return carry

    lax.fori_loop(0, H * NB, body, 0)


def _attention(k_ref, qt_ref, vt_ref, ot_ref, kb_ref, z_ref, pc_ref, ac_ref, bias_ref,
               vflag_ref, sliding):
    if sliding:
        bad = _sliding_attention(k_ref, qt_ref, vt_ref, ot_ref, z_ref, pc_ref, ac_ref, bias_ref)
    else:
        bad = _full_attention(k_ref, qt_ref, vt_ref, ot_ref, kb_ref, z_ref, pc_ref, ac_ref)

    bad = jnp.maximum(bad, jnp.max(vflag_ref[...].reshape(S // TM * 8, TM), axis=0, keepdims=True))

    @pl.when(jnp.max(bad) > 0.0)
    def _():
        _safe_attention(k_ref, qt_ref, vt_ref, ot_ref, sliding)


def _layernorm(x):
    m = jnp.mean(x, axis=-1, keepdims=True)
    xc = x - m
    v = jnp.mean(xc * xc, axis=-1, keepdims=True)
    return (xc * lax.rsqrt(v + LN_EPS)).astype(BF16)


def _project_k(xn, i, wk, k_ref, g0=0, copies=NP):
    k = _swap8(jnp.dot(xn, wk, preferred_element_type=F32))
    for g in range(wk.shape[1] // LANE):
        kg = _pk(k[:, g * LANE:(g + 1) * LANE].astype(BF16))
        for p in range(copies):
            k_ref[(g0 + g) * NP + p, pl.ds(_mo(i * (TM // 2), TM // 2), TM // 2), :] = (
                pltpu.roll(kg, LANE - p * HPI * DH, 1) if p else kg)


def _project_qv(xn, i, wt, qt_ref, vt_ref, vflag_ref):
    qv = lax.dot_general(wt, xn, (((1,), (1,)), ((), ())),
                         preferred_element_type=F32)
    for t in range(TM // LANE):
        j = i * (TM // LANE) + t
        qt = _pk((qv[:D, t * LANE:(t + 1) * LANE] * QSCALE).astype(BF16))
        vt = _pk(qv[D:, t * LANE:(t + 1) * LANE].astype(BF16))
        r = pl.ds(_mo(j * PR, PR), PR)
        for p in range(H // HPI):
            qt_ref[p, r, :] = qt[p * PR:(p + 1) * PR]
            vt_ref[p, r, :] = vt[p * PR:(p + 1) * PR]
    big = jnp.where(jnp.abs(qv[D:]) < V_HI, 0.0, 1.0)
    vflag_ref[i] = jnp.max(big.reshape(D // 8, 8, TM), axis=0)


def _project_out(i, ot_ref, wo, tm=TM):
    ot = _unpk(_cat([_cat([ot_ref[p, pl.ds(_mo((i * (tm // LANE) + t) * PR, PR), PR), :]
                           for p in range(H // HPI)], 0)
                     for t in range(tm // LANE)], 1))
    return lax.dot_general(ot, wo, (((0,), (0,)), ((), ())),
                           preferred_element_type=F32)


def _kernel(x_hbm, wa_hbm, woa_hbm, wb_hbm, wob_hbm, o_hbm,
            xb_ref, w_ref, wo_ref, wt_ref, xres_ref, xn_ref,
            k_ref, qt_ref, vt_ref, ot_ref, kb_ref, z_ref, pc_ref, ac_ref, bias_ref, vflag_ref, sems):
    nchunk = S // TM

    def rows(i):
        return pl.ds(_mo(i * TM, TM), TM)

    x_cp = [pltpu.make_async_copy(x_hbm.at[rows(i)], xb_ref.at[rows(i)], sems.at[i])
            for i in range(nchunk)]
    wa_cp = [pltpu.make_async_copy(wa_hbm.at[:, pl.ds(n * D, D)], w_ref.at[0, n],
                                   sems.at[nchunk + n]) for n in range(3)]
    wb_cp = [pltpu.make_async_copy(wb_hbm.at[:, pl.ds(n * D, D)], w_ref.at[1, n],
                                   sems.at[nchunk + 3 + n]) for n in range(3)]
    wo_cp = [pltpu.make_async_copy(src, wo_ref.at[n], sems.at[nchunk + 6 + n])
             for n, src in enumerate((woa_hbm, wob_hbm))]
    for cp in (x_cp[0], wa_cp[1], *x_cp[1:], wa_cp[0], wa_cp[2],
               wb_cp[0], wb_cp[2], wb_cp[1], *wo_cp):
        cp.start()

    z_ref[...] = jnp.zeros(z_ref.shape, F32)
    _init_bias(bias_ref)
    _init_carry(pc_ref, ac_ref)

    def normalize(i, x):
        xres_ref[rows(i), :] = x
        return _layernorm(x)

    def project_qv(i, xn, kind):
        _project_qv(xn, i, _unpk(wt_ref[kind]), qt_ref, vt_ref, vflag_ref)

    def stash(i):
        xn = normalize(i, xb_ref[rows(i), :].astype(F32))
        xn_ref[i] = _pk(xn)
        return xn

    def first_k(xn, i, half):
        _project_k(xn, i, w_ref[0, 1, :, half * (D // 2):(half + 1) * (D // 2)], k_ref,
                   half * (NG // 2), 1)

    x_cp[0].wait()
    xn0 = stash(0)
    wa_cp[1].wait()
    first_k(xn0, 0, 0)
    x_cp[1].wait()
    first_k(xn0, 0, 1)
    xn1 = stash(1)
    first_k(xn1, 1, 0)
    x_cp[2].wait()
    x_cp[3].wait()
    first_k(xn1, 1, 1)
    xn2 = stash(2)
    _project_k(xn2, 2, w_ref[0, 1], k_ref, 0, 1)
    xn3 = stash(3)
    first_k(xn3, 3, 0)
    wa_cp[0].wait()
    wa_cp[2].wait()
    first_k(xn3, 3, 1)
    wt_ref[0, 0:D // 2, :] = _pk(w_ref[0, 0].T)
    wt_ref[0, D // 2:D, :] = _pk(w_ref[0, 2].T)

    def first_qv(it, c):
        n = 2 * it
        pltpu.make_async_copy(wb_hbm.at[:, pl.ds(pl.multiple_of(n * D, D), D)],
                              w_ref.at[1, n], sems.at[nchunk + 3 + n]).wait()
        for i in (2 * it, 2 * it + 1):
            project_qv(i, _unpk(xn_ref[i]), 0)
        r = pl.ds(pl.multiple_of(it * TM, TM), TM)
        for g in range(NG):
            kg = k_ref[g * NP, r, :]
            for p in range(1, NP):
                k_ref[g * NP + p, r, :] = pltpu.roll(kg, LANE - p * HPI * DH, 1)
        wt_ref[1, pl.ds(pl.multiple_of(it * (D // 2), D // 2), D // 2), :] = _pk(w_ref[1, n].T)
        return c

    lax.fori_loop(0, 2, first_qv, 0)
    for cp in (wb_cp[1], *wo_cp):
        cp.wait()

    def layer(t, carry):
        cur = t & 1

        @pl.when(cur == 0)
        def _():
            _attention(k_ref, qt_ref, vt_ref, ot_ref, kb_ref, z_ref, pc_ref, ac_ref, bias_ref,
                       vflag_ref, sliding=True)

        @pl.when(cur == 1)
        def _():
            _attention(k_ref, qt_ref, vt_ref, ot_ref, kb_ref, z_ref, pc_ref, ac_ref, bias_ref,
                       vflag_ref, sliding=False)

        @pl.when(t < 3)
        def _():
            nxt = 1 - cur

            def resid(i):
                xns = []
                for m in range(TM // TR):
                    r = pl.ds(pl.multiple_of(i * TM + m * TR, TR), TR)
                    x = xres_ref[r, :] + _project_out(i * (TM // TR) + m, ot_ref, wo_ref[cur], TR)
                    xres_ref[r, :] = x
                    xns.append(_layernorm(x))
                return _cat(xns, 0)

            def half(it, c):
                a, b = 2 * it, 2 * it + 1
                xa = resid(a)
                xb = resid(b)
                _project_k(xa, a, w_ref[nxt, 1], k_ref)
                _project_k(xb, b, w_ref[nxt, 1], k_ref)
                project_qv(a, xa, nxt)
                project_qv(b, xb, nxt)
                for u in range(HPI):
                    _prep_kb(0, u, k_ref, kb_ref, it)
                _init_carry(pc_ref, ac_ref)
                return c

            lax.fori_loop(0, nchunk // 2, half, 0)
        return carry

    lax.fori_loop(0, 4, layer, 0)

    o_cp = [pltpu.make_async_copy(xb_ref.at[pl.ds(i * TR, TR)], o_hbm.at[pl.ds(i * TR, TR)],
                                  sems.at[i]) for i in range(S // TR)]
    for i in range(S // TR):
        x = xres_ref[pl.ds(i * TR, TR), :] + _project_out(i, ot_ref, wo_ref[1], TR)
        xb_ref[pl.ds(i * TR, TR), :] = x.astype(BF16)
        o_cp[i].start()
    for cp in o_cp:
        cp.wait()


@jax.jit
def pallas_interleave_layers__sliding_block__mha_block__prompt_kernel(
    A_x: jax.Array,
    A_wqkv: jax.Array,
    A_wo: jax.Array,
    B_x: jax.Array,
    B_wqkv: jax.Array,
    B_wo: jax.Array,
):
    del B_x
    x = A_x.reshape(S, D)
    any_spec = pl.BlockSpec(memory_space=pl.ANY)
    out = pl.pallas_call(
        _kernel,
        out_shape=jax.ShapeDtypeStruct((S, D), A_x.dtype),
        in_specs=[any_spec] * 5,
        out_specs=any_spec,
        scratch_shapes=[
            pltpu.VMEM((S, D), BF16),
            pltpu.VMEM((2, 3, D, D), BF16),
            pltpu.VMEM((2, D, D), BF16),
            pltpu.VMEM((2, D, D), U32),
            pltpu.VMEM((S, D), F32),
            pltpu.VMEM((S // TM, TM // 2, D), U32),
            pltpu.VMEM((NG * NP, S // 2, LANE), U32),
            pltpu.VMEM((H // HPI, NB * PR, LANE), U32),
            pltpu.VMEM((H // HPI, NB * PR, LANE), U32),
            pltpu.VMEM((H // HPI, NB * PR, LANE), U32),
            pltpu.VMEM((HPI, DH, 2 * KB_HALF * RV // 2, LANE), U32),
            pltpu.VMEM((DH, 4 * LANE), F32),
            pltpu.VMEM((3, LANE // 2, 4 * LANE), U32),
            pltpu.VMEM((DH + 8, 4 * LANE), F32),
            pltpu.VMEM((2, LANE, LANE), F32),
            pltpu.VMEM((S // TM, 8, TM), F32),
            pltpu.SemaphoreType.DMA((max(S // TM + 8, S // TR),)),
        ],
        compiler_params=pltpu.CompilerParams(vmem_limit_bytes=100 * 1024 * 1024),
    )(x, A_wqkv, A_wo, B_wqkv, B_wo)
    return out.reshape(A_x.shape)
```
